```python
import os as _os
_os.environ.setdefault("JAX_PLATFORMS", "cpu")
import jax
import jax.numpy as jnp

def _softmax(x, axis=-1):
    return jax.nn.softmax(x, axis=axis)
def _gelu(x):
    return jax.nn.gelu(x, approximate=True)
def _silu(x):
    return jax.nn.silu(x)
def _sigmoid(x):
    return jax.nn.sigmoid(x)
def _layernorm(x, axis=-1, eps=1e-5):
    m = jnp.mean(x, axis=axis, keepdims=True)
    v = jnp.var(x, axis=axis, keepdims=True)
    return (x - m) / jnp.sqrt(v + eps)
def _scatter_add(tgt, idx, src, axis=0):
    return tgt.at[idx].add(src)
def _segment_sum(src, seg, n):
    return jax.ops.segment_sum(src, seg, n)
class _Rng:
    def __init__(self, key):
        self._k = key
    def _next(self):
        self._k, sub = jax.random.split(self._k)
        return sub
    def normal(self, shape):
        return jax.random.normal(self._next(), shape, dtype=jnp.bfloat16)
    def randint(self, lo, hi, shape):
        return jax.random.randint(self._next(), shape, lo, hi, dtype=jnp.int32)
    def uniform(self, shape, lo=0.0, hi=1.0):
        return jax.random.uniform(self._next(), shape, jnp.bfloat16, lo, hi)
    def permutation(self, n):
        return jax.random.permutation(self._next(), n)


kernel_name = 'sequential_preLN__softmax_full_mha__dense_activation_squared_relu__prompt'

def setup_inputs():
    _rng = _Rng(jax.random.key(int.from_bytes(__import__("os").urandom(4), "little")))
    _w = (lambda a: (lambda t: t.astype(jnp.bfloat16) if jnp.issubdtype(t.dtype, jnp.floating) else t)(jnp.asarray(a)))
    def _A_setup():
        B, S, D = 1, 2048, 640
        return {
            "x": _w((lambda *s: _rng.normal(s) * 0.05)(B, S, D)),
            "wqkv": _w((lambda *s: _rng.normal(s) * 0.05)(D, 3 * D)),
            "wo": _w((lambda *s: _rng.normal(s) * 0.05)(D, D)),
        }
    _A_in = _A_setup()

    def _B_setup():
        B, S, D, F = 1, 2048, 640, 1536
        return {
            "x": _w((lambda *s: _rng.normal(s) * 0.05)(B, S, D)),
            "w1": _w((lambda *s: _rng.normal(s) * 0.05)(D, F)),
            "b1": _w((lambda *s: _rng.normal(s) * 0.05)(F)),
            "w2": _w((lambda *s: _rng.normal(s) * 0.05)(F, D)),
            "b2": _w((lambda *s: _rng.normal(s) * 0.05)(D)),
        }
    _B_in = _B_setup()

    return {
        "A_x": _A_in["x"],
        "A_wqkv": _A_in["wqkv"],
        "A_wo": _A_in["wo"],
        "B_x": _B_in["x"],
        "B_w1": _B_in["w1"],
        "B_b1": _B_in["b1"],
        "B_w2": _B_in["w2"],
        "B_b2": _B_in["b2"],
    }

def reference(A_x, A_wqkv, A_wo, B_x, B_w1, B_b1, B_w2, B_b2):
    def _A_ref(x, wqkv, wo):
        B, S, D = x.shape
        H = 32; Dh = D // H
        qkv = (lambda x, *d: x.transpose(*d))((x @ wqkv).reshape(B, S, 3, H, Dh), 2, 0, 3, 1, 4)
        q, k, v = qkv[0], qkv[1], qkv[2]
        scale = Dh ** -0.5
        scores = jnp.einsum("bhqd,bhkd->bhqk", q, k) * scale
        p = _softmax(scores, axis=-1)
        o = jnp.einsum("bhqk,bhkd->bhqd", p, v)
        return (lambda x, *d: x.transpose(*d))(o, 0, 2, 1, 3).reshape(B, S, D) @ wo

    def _B_ref(x, w1, b1, w2, b2):
        h = jnp.einsum("bsd,df->bsf", x, w1) + b1
        zero = jnp.zeros_like(h)
        r = jnp.where(h > zero, h, zero)
        h = r * r
        out = jnp.einsum("bsf,fd->bsd", h, w2) + b2
        return out

    x = A_x
    h = x + _A_ref(_layernorm(x, axis=-1), A_wqkv, A_wo)
    h2 = h + _B_ref(_layernorm(h, axis=-1), B_w1, B_b1, B_w2, B_b2)
    return h2
```

```python
import functools
import jax
import jax.numpy as jnp
from jax import lax
import jax.experimental.pallas as pl
import jax.experimental.pallas.tpu as pltpu

F32, BF16, U32 = jnp.float32, jnp.bfloat16, jnp.uint32
LOG2E = 1.4426950408889634
NT = (((1,), (1,)), ((), ()))
TN = (((0,), (0,)), ((), ()))


def _unpack(x):
    return pltpu.bitcast(x, BF16)


def _pack(x):
    return pltpu.bitcast(x.astype(BF16), U32)


def _layernorm(x):
    m = jnp.mean(x, axis=-1, keepdims=True)
    d = x - m
    v = jnp.mean(d * d, axis=-1, keepdims=True)
    return d * lax.rsqrt(v + 1e-5)


def make(S=2048, D=640, H=32, F=1536, TQ=512, C=256, TB=512, PAIRS_PER_ITER=1):
    Dh = D // H
    NQ = S // TQ
    NP = H // 2
    NB = D // 128

    def kernel(x_hbm, wqkv_hbm, wo_hbm, w1_hbm, b1_ref, w2_hbm, b2_ref, o_hbm,
               x_v, wqkv_v, wo_v, w1_v, w2_v, o_v,
               wt_s, k_s, qt_s, vt_s, ot_s, s_s, m_s, sems):
        nblk = S // TB
        cp_x = [pltpu.make_async_copy(x_hbm.at[0, pl.ds(i * TB, TB)], x_v.at[pl.ds(i * TB, TB)], sems.at[i]) for i in range(nblk)]
        cp_wqkv = pltpu.make_async_copy(wqkv_hbm, wqkv_v, sems.at[nblk])
        cp_wo = pltpu.make_async_copy(wo_hbm, wo_v, sems.at[nblk + 1])
        cp_w1 = pltpu.make_async_copy(w1_hbm, w1_v, sems.at[nblk + 2])
        cp_w2 = pltpu.make_async_copy(w2_hbm, w2_v, sems.at[nblk + 3])
        cp_o = [pltpu.make_async_copy(o_v.at[pl.ds(i * TB, TB)], o_hbm.at[0, pl.ds(i * TB, TB)], sems.at[nblk + 4 + i]) for i in range(nblk)]
        cp_x[0].start()
        cp_wqkv.start()
        for c in cp_x[1:]:
            c.start()
        cp_wo.start(); cp_w1.start(); cp_w2.start()

        cp_wqkv.wait()
        wt_s[0:D // 2] = pltpu.bitcast(wqkv_v[:, 0:D].T, U32)
        wt_s[D // 2:D] = pltpu.bitcast(wqkv_v[:, 2 * D:3 * D].T, U32)
        lane = lax.broadcasted_iota(jnp.int32, (TB // 2, 128), 1)
        for i in range(nblk):
            cp_x[i].wait()
            xn = _layernorm(x_v[i * TB:(i + 1) * TB, :].astype(F32)).astype(BF16)
            k = _pack(jnp.dot(xn, wqkv_v[:, D:2 * D], preferred_element_type=F32))
            rows = slice(i * TB // 2, (i + 1) * TB // 2)
            for b in range(NB):
                k_s[b, rows, :] = k[:, b * 128:(b + 1) * 128]
            for b in range(NB - 1):
                k_s[NB + b, rows, :] = jnp.where(lane < 64, k[:, (b + 1) * 128:(b + 2) * 128], k[:, b * 128:(b + 1) * 128])
            qv = lax.dot_general(_unpack(wt_s[...]), xn, NT, preferred_element_type=F32)
            q = _pack(qv[0:D] * (Dh ** -0.5 * LOG2E))
            v = qv[D:2 * D].astype(BF16).astype(F32)
            for u in range(TB // TQ):
                qt_s[i * (TB // TQ) + u] = q[:, u * TQ:(u + 1) * TQ].reshape(NB, 64, TQ)
            vt_s[:, :, i * TB:(i + 1) * TB] = v.reshape(NP, 2 * Dh, TB)

        row64 = lax.broadcasted_iota(jnp.int32, (64, TQ), 0)
        sub = lax.broadcasted_iota(jnp.int32, (8, C), 0)
        subq = lax.broadcasted_iota(jnp.int32, (8, TQ), 0)

        def masked_q(qb, h):
            lo = (Dh // 2) * h
            b0 = lo // 64
            b1 = (lo + Dh // 2 - 1) // 64
            g0 = row64 + b0 * 64 - lo
            g1 = row64 + b1 * 64 - lo
            m0 = (g0 >= 0) & (g0 < Dh // 2)
            m1 = (g1 >= 0) & (g1 < Dh // 2)
            qm = jnp.where(m0, qt_s[qb, b0], jnp.where(m1, qt_s[qb, b1], jnp.uint32(0)))
            return _unpack(qm), jnp.where(b0 == b1, b0, NB + b0)

        def step(ta, tb):
            outs = []
            for e in range(2):
                if ta is not None:
                    qm, kv = masked_q(ta // NP, 2 * (ta % NP) + e)
                    m_new = None
                if tb is not None:
                    jb = tb % NP
                    m_old = m_s[e]
                    acc = None
                for c in range(S // C):
                    rows = slice(c * C, (c + 1) * C)
                    if tb is not None:
                        s = s_s[e, rows, :]
                        p = jnp.exp2(s.reshape(C // 8, 8, TQ) - m_old[None]).reshape(C, TQ).astype(BF16)
                        if e == 0:
                            vt = jnp.concatenate([vt_s[jb, 0:16, rows], jnp.where(sub < 4, vt_s[jb, 16:24, rows], 1.0)], axis=0)
                        else:
                            vt = jnp.concatenate([jnp.where(sub >= 4, vt_s[jb, 16:24, rows], 1.0), vt_s[jb, 24:40, rows]], axis=0)
                        pv = jnp.dot(vt, p, preferred_element_type=F32)
                        acc = pv if acc is None else acc + pv
                    if ta is not None:
                        s = jnp.dot(_unpack(k_s[kv, c * C // 2:(c + 1) * C // 2, :]), qm, preferred_element_type=F32)
                        s_s[e, rows, :] = s
                        mc = jnp.max(s.reshape(C // 8, 8, TQ), axis=0)
                        m_new = mc if m_new is None else jnp.maximum(m_new, mc)
                if ta is not None:
                    m_s[e] = jnp.broadcast_to(jnp.max(m_new, axis=0, keepdims=True), (8, TQ))
                if tb is not None:
                    l = acc[23:24] if e == 0 else acc[0:1]
                    outs.append(acc * (1.0 / l))
            if tb is not None:
                qb, jb = tb // NP, tb % NP
                mid = jnp.where(subq < 4, outs[0][16:24], outs[1][0:8])
                ot_s[qb, jb] = jnp.concatenate([outs[0][0:16], mid, outs[1][8:24]], axis=0)

        n_items = NQ * NP
        step(0, None)

        def body(t, carry):
            for u in range(PAIRS_PER_ITER):
                tt = 1 + t * PAIRS_PER_ITER + u
                step(tt, tt - 1)
            return carry
        n_loop = (n_items - 1) // PAIRS_PER_ITER
        lax.fori_loop(0, n_loop, body, 0)
        for tt in range(1 + n_loop * PAIRS_PER_ITER, n_items):
            step(tt, tt - 1)
        step(None, n_items - 1)

        cp_wo.wait(); cp_w1.wait(); cp_w2.wait()
        b1 = b1_ref[...].astype(F32).reshape(1, F)
        b2 = b2_ref[...].astype(F32).reshape(1, D)
        for i in range(nblk):
            rows = slice(i * TB, (i + 1) * TB)
            ot = jnp.concatenate([ot_s[i * (TB // TQ) + u].reshape(D, TQ) for u in range(TB // TQ)], axis=1)
            a = lax.dot_general(ot.astype(BF16), wo_v[...], TN, preferred_element_type=F32)
            h = x_v[rows, :].astype(F32) + a
            hn = _layernorm(h).astype(BF16)
            g = jnp.dot(hn, w1_v[...], preferred_element_type=F32) + b1
            r = jnp.maximum(g, 0.0)
            y = jnp.dot((r * r).astype(BF16), w2_v[...], preferred_element_type=F32)
            o_v[rows, :] = (h + (y + b2)).astype(BF16)
            cp_o[i].start()
        for c in cp_o:
            c.wait()

    @jax.jit
    def run(A_x, A_wqkv, A_wo, B_x, B_w1, B_b1, B_w2, B_b2):
        del B_x
        anyspec = pl.BlockSpec(memory_space=pl.ANY)
        vmem = pl.BlockSpec(memory_space=pltpu.VMEM)
        return pl.pallas_call(
            kernel,
            out_shape=jax.ShapeDtypeStruct((1, S, D), BF16),
            in_specs=[anyspec, anyspec, anyspec, anyspec, vmem, anyspec, vmem],
            out_specs=anyspec,
            scratch_shapes=[
                pltpu.VMEM((S, D), BF16), pltpu.VMEM((D, 3 * D), BF16), pltpu.VMEM((D, D), BF16),
                pltpu.VMEM((D, F), BF16), pltpu.VMEM((F, D), BF16), pltpu.VMEM((S, D), BF16),
                pltpu.VMEM((D, D), U32),
                pltpu.VMEM((2 * NB - 1, S // 2, 128), U32),
                pltpu.VMEM((NQ, NB, 64, TQ), U32),
                pltpu.VMEM((NP, 2 * Dh, S), F32),
                pltpu.VMEM((NQ, NP, 2 * Dh, TQ), F32),
                pltpu.VMEM((2, S, TQ), F32),
                pltpu.VMEM((2, 8, TQ), F32),
                pltpu.SemaphoreType.DMA((2 * (S // TB) + 4,)),
            ],
            compiler_params=pltpu.CompilerParams(vmem_limit_bytes=110 * 2**20),
        )(A_x, A_wqkv, A_wo, B_w1, B_b1, B_w2, B_b2)
    return run


_run = make()


def pallas_sequential_preLN__softmax_full_mha__dense_activation_squared_relu__prompt_kernel(A_x, A_wqkv, A_wo, B_x, B_w1, B_b1, B_w2, B_b2):
    return _run(A_x, A_wqkv, A_wo, B_x, B_w1, B_b1, B_w2, B_b2)
```

```python
import functools
import numpy as np
import jax
import jax.numpy as jnp
from jax import lax
import jax.experimental.pallas as pl
import jax.experimental.pallas.tpu as pltpu

F32, BF16, U32 = jnp.float32, jnp.bfloat16, jnp.uint32
LOG2E = 1.4426950408889634
L_MIN, L_MAX, O_MAX = 2.0 ** -60, 2.0 ** 100, 2.0 ** 120


def _as_bf16(x):
    return pltpu.bitcast(x, BF16)


def _as_u32(x):
    return pltpu.bitcast(x, U32)


def _spread(jobs, n):
    cut = [(i * len(jobs)) // n for i in range(n + 1)]
    return [jobs[cut[i]:cut[i + 1]] for i in range(n)]


def make(S=2048, D=640, H=32, F=1536, TQ=512, pattern=(2,), phases=(1, 2, 3), fallback=True, flags=None,
         seg=2, mem=True, pad=4, strassen=(1, 1, 1, 1), ties=True, R1=64, scopes=False, w_cuts=(0, 1, 6, 15), ln_at=5, defer=True, RP=16, early=1, lead=8, delay=0):
    Dh = D // H
    NQ, NP, NB, NC, NL = S // TQ, H // 2, D // 128, S // 128, TQ // 128
    TB = 2 * TQ
    NT = S // TB
    KH = (D // 256) * 128
    G = [pattern[c % len(pattern)] for c in range(NC)]
    GM = max(max(G), 1)
    goff = [int(v) for v in np.cumsum([0] + G)]
    NG = goff[-1]
    NVB = -(-NG // 16)
    KB0, KW0 = 0, NG * Dh
    PV0 = KW0 + NC * 8
    NPV = 64
    AC0 = PV0 + NPV
    NY = AC0 + 1

    def kernel(z_ref, x_hbm, wqkv_hbm, wo_hbm, w1_hbm, b1_ref, w2_hbm, b2_ref, o_hbm,
               x_v, wqkv_v, wo_v, w1_v, w2_v, o_v,
               xt_s, qt_s, kt_s, vt_s, ot_s, kv_s, y_s, aq_s, a_s, b_s, c_s, bias_s, sem_x, sem_w, sems):
        zero = z_ref[0]
        sub = lax.broadcasted_iota(jnp.int32, (8, 128), 0)
        lane = lax.broadcasted_iota(jnp.int32, (8, 128), 1)
        always = (sub + zero) >= 0

        x_cuts = [128 * i for i in range(2 * NL + 1)] + [S]
        cp_x = [pltpu.make_async_copy(x_hbm.at[0, pl.ds(a, b - a)], x_v.at[pl.ds(a, b - a)], sem_x.at[i])
                for i, (a, b) in enumerate(zip(x_cuts, x_cuts[1:]))]
        cp_w = [pltpu.make_async_copy(wqkv_hbm.at[:, pl.ds(128 * a, 128 * (b - a))], wqkv_v.at[:, pl.ds(128 * a, 128 * (b - a))], sem_w.at[i])
                for i, (a, b) in enumerate(zip(w_cuts, w_cuts[1:]))]
        cp_wo = pltpu.make_async_copy(wo_hbm, wo_v, sems.at[0])
        cp_w1 = pltpu.make_async_copy(w1_hbm, w1_v, sems.at[1])
        cp_w2 = pltpu.make_async_copy(w2_hbm, w2_v, sems.at[2])
        cp_o = [[pltpu.make_async_copy(o_v.at[t * NB + r],
                                       o_hbm.at[0, pl.ds(t * TB, TB), pl.ds(r * 128, 128)],
                                       sems.at[3 + t * NB + r]) for r in range(NB)] for t in range(NT)]

        def mark(name, fn):
            if scopes:
                with jax.named_scope(name):
                    fn()
            else:
                fn()

        def rows_get(ref, r0, n, cols):
            return jnp.concatenate([ref[i // 5, 8 * (i % 5):8 * (i % 5) + 8, cols] for i in range(r0 // 8, (r0 + n) // 8)], axis=0)

        def rows_put(ref, r0, val, cols):
            for k in range(val.shape[0] // 8):
                i = r0 // 8 + k
                ref[i // 5, 8 * (i % 5):8 * (i % 5) + 8, cols] = val[8 * k:8 * k + 8]

        def groups(v):
            return [v[8 * i:8 * i + 8, 128 * k:128 * k + 128] for k in range(v.shape[1] // 128) for i in range(v.shape[0] // 8)]

        def after(val, jobs):
            deps = [pltpu.bitcast(v, F32) for job in jobs for v in job()]
            if not deps or not ties:
                return val
            nr = val.shape[0] // 8
            tiles = groups(val)
            for i, vs in enumerate(_spread(deps, len(tiles))):
                for v in vs:
                    tiles[i] = jnp.where(always, tiles[i], v)
            return jnp.concatenate([jnp.concatenate(tiles[i::nr], axis=1) for i in range(nr)], axis=0)

        def left_operand(use_strassen, i, blk):
            f = lambda u: blk(u).astype(F32)
            if not use_strassen:
                return blk(i)
            return (lambda: (f(0) + f(3)).astype(BF16), lambda: (f(2) + f(3)).astype(BF16), lambda: blk(0), lambda: blk(3),
                    lambda: (f(0) + f(1)).astype(BF16), lambda: (f(2) - f(0)).astype(BF16), lambda: (f(1) - f(3)).astype(BF16))[i]()

        def right_operand(use_strassen, i, blk):
            if not use_strassen:
                return blk(i).astype(BF16)
            return (lambda: blk(0) + blk(3), lambda: blk(0), lambda: blk(1) - blk(3), lambda: blk(2) - blk(0),
                    lambda: blk(3), lambda: blk(0) + blk(1), lambda: blk(2) + blk(3))[i]().astype(BF16)

        def block_product(use_strassen, a, ar, b, br, jobs=()):
            n = (7 if use_strassen else 8) + (4 if ar is not None else 0)
            js = iter(_spread(list(jobs), n))
            mm = lambda l, r: after(jnp.dot(l, r, preferred_element_type=F32), next(js))
            rest = (lambda c, i, k: c + mm(ar(i), br(k))) if ar is not None else (lambda c, i, k: c)
            if not use_strassen:
                return [[rest(mm(a(2 * i), b(k)) + mm(a(2 * i + 1), b(2 + k)), i, k) for k in range(2)] for i in range(2)]
            m = lambda i: mm(a(i), b(i))
            m1 = m(0)
            m4 = m(3)
            m5 = m(4)
            c11 = rest(m1 + m4 - m5 + m(6), 0, 0)
            m2 = m(1)
            c21 = rest(m2 + m4, 1, 0)
            m3 = m(2)
            c12 = rest(m3 + m5, 0, 1)
            c22 = rest(m1 - m2 + m3 + m(5), 1, 1)
            return [[c11, c12], [c21, c22]]

        def weight_jobs(use_strassen, a_ref, base, rows, kh, nrest, top, bot):
            nk = kh // 128
            memo = {}

            def blk(u):
                if not memo:
                    memo[0] = (top(), bot())
                return memo[0][u // 2][:, (u % 2) * kh:(u % 2 + 1) * kh]

            def main(i):
                v = _as_u32(left_operand(use_strassen, i, blk))
                for k in range(nk):
                    a_ref[zero + (base + i * nk + k), 0:rows // 2] = v[:, 128 * k:128 * k + 128]
                return groups(v)

            def rest(i):
                blk(0)
                v = _as_u32(memo[0][i][:, 2 * kh:])
                a_ref[zero + (base + 7 * nk + i), 0:rows // 2] = v
                return groups(v)
            return [functools.partial(main, i) for i in range(7 if use_strassen else 4)] + [functools.partial(rest, i) for i in range(nrest)]

        def weight_operands(a_ref, base, rows, kh):
            nk = kh // 128
            a = lambda i: _as_bf16(jnp.concatenate([a_ref[base + i * nk + k, 0:rows // 2] for k in range(nk)], axis=1))
            return a, (lambda i: _as_bf16(a_ref[base + 7 * nk + i, 0:rows // 2]))

        def halves(load):
            memo = {}

            def wt():
                if not memo:
                    memo[0] = load().T
                return memo[0]
            return (lambda: wt()[0:64]), (lambda: wt()[64:128])

        def right_jobs(use_strassen, slot, l, rows):
            def main(r0):
                blk = [rows(u % 2, (u // 2) * KH + r0, RP) for u in range(4)]
                out = []
                for i in range(7 if use_strassen else 4):
                    v = _as_u32(right_operand(use_strassen, i, lambda u: blk[u]))
                    b_s[slot][zero + i, r0 // 2:(r0 + RP) // 2, 128 * l:128 * l + 128] = v
                    out += groups(v)
                return out

            def rest(k):
                v = _as_u32(rows(k, 2 * KH, D - 2 * KH).astype(BF16))
                b_s[slot][zero + 7, 64 * k:64 * k + 64, 128 * l:128 * l + 128] = v
                return groups(v)
            return [functools.partial(main, r0) for r0 in range(0, KH, RP)] + [functools.partial(rest, k) for k in range(2)]

        def get_right(slot):
            return (lambda i: _as_bf16(b_s[slot][i])), (lambda k: _as_bf16(b_s[slot][7, 64 * k:64 * k + 64]))

        def norm_jobs(use_strassen, t, l, slot, from_x):
            tile = [k * NL + l for k in range(2)]
            mean, rstd = {}, {}

            part = {}

            def add_tiles(key, v):
                v = [v[8 * i:8 * i + 8] for i in range(v.shape[0] // 8)] + ([part[key]] if key in part else [])
                while len(v) > 1:
                    v = [v[i] + v[i + 1] for i in range(0, len(v) - 1, 2)] + v[len(v) - len(v) % 2:]
                part[key] = v[0]
                return v

            def mean_job(k, b):
                rr = slice(128 * b, 128 * b + 128)
                if from_x:
                    v = x_v[t * TB + tile[k] * 128:t * TB + (tile[k] + 1) * 128, rr].T.astype(F32)
                    xt_s[t][zero + tile[k], rr] = v
                else:
                    v = xt_s[t][tile[k], rr]
                out = add_tiles(("sum", k), v)
                if b == NB - 1:
                    mean[k] = jnp.broadcast_to(jnp.sum(out[0], axis=0, keepdims=True) * (1.0 / D), (8, 128))
                    out = [mean[k]]
                return out

            def centered(k, r0, n):
                return (xt_s[t][zero + tile[k], r0:r0 + n].reshape(n // 8, 8, 128) - mean[k][None]).reshape(n, 128)

            def var_job(k, b):
                d = centered(k, 128 * b, 128)
                out = add_tiles(("var", k), d * d)
                if b == NB - 1:
                    rstd[k] = jnp.broadcast_to(lax.rsqrt(jnp.sum(out[0], axis=0, keepdims=True) * (1.0 / D) + 1e-5), (8, 128))
                    out = [rstd[k]]
                return out
            memo = {}

            def rows(k, r0, n):
                if (k, r0) not in memo:
                    memo[(k, r0)] = (centered(k, r0, n).reshape(n // 8, 8, 128) * rstd[k][None]).reshape(n, 128)
                return memo[(k, r0)]
            return ([functools.partial(job, k, b) for job in (mean_job, var_job) for k in range(2) for b in range(NB)]
                    + right_jobs(use_strassen, slot, l, rows))

        NF = F // (2 * R1)
        A_O, A_1 = 0, 16 * NB
        A_2 = A_1 + 16 * NF

        def w2_slab(r):
            w = w2_v[:, 128 * r:128 * r + 128]
            return jnp.concatenate([w[2 * R1 * q + R1 * i:2 * R1 * q + R1 * (i + 1)] for i in range(2) for q in range(NF)], axis=0)

        qkv_jobs = [weight_jobs(strassen[0], aq_s[r % 2], 16 * (r // 2), 64, KH, 2, *halves(lambda r=r: wqkv_v[:, 128 * r:128 * r + 128])) for r in range(3 * NB)]
        tail_jobs = []
        for r in range(NB):
            tail_jobs += weight_jobs(strassen[1], a_s, A_O + 16 * r, 64, KH, 2, *halves(lambda r=r: wo_v[:, 128 * r:128 * r + 128]))
        for r in range(NF):
            tail_jobs += weight_jobs(strassen[2], a_s, A_1 + 16 * r, R1, KH, 2,
                                     lambda r=r: w1_v[:, 2 * R1 * r:2 * R1 * r + R1].T, lambda r=r: w1_v[:, 2 * R1 * r + R1:2 * R1 * (r + 1)].T)
        for r in range(NB):
            tail_jobs += weight_jobs(strassen[3], a_s, A_2 + 7 * (F // 256) * r, 64, F // 2, 0, *halves(functools.partial(w2_slab, r)))

        def bias_job(ref, n, base, r):
            bias = ref[...].astype(F32).reshape(1, n)
            v = jnp.broadcast_to(bias[:, 128 * r:128 * r + 128], (128, 128)).T
            bias_s[base + 128 * r:base + 128 * r + 128, :] = v
            return groups(v)
        if 3 in phases:
          tail_jobs += [functools.partial(bias_job, ref, n, base, r) for ref, base, n in ((b1_ref, 0, F), (b2_ref, F, D)) for r in range(n // 128)]

        def gather_job(i):
            p, rr = i // 5, slice(8 * (i % 5), 8 * (i % 5) + 8)
            out = []
            for beta in range(NVB):
                acc = jnp.zeros((8, 128), F32)
                for c in range(NC):
                    lo, hi = max(8 * goff[c], 128 * beta), min(8 * goff[c + 1], 128 * beta + 128)
                    if lo < hi:
                        src = 128 - 8 * G[c] + lo - 8 * goff[c]
                        v = kt_s[zero + p, rr, 128 * c:128 * c + 128]
                        shift = (lo - 128 * beta - src) % 128
                        v = pltpu.roll(v, shift, 1) if shift else v
                        acc = jnp.where((lane >= lo - 128 * beta) & (lane < hi - 128 * beta), v, acc)
                kv_s[p, rr, 128 * beta:128 * beta + 128] = acc
                out.append(acc)
            return out

        def k_window(j, e, cols):
            return kt_s[j, 8 * e:8 * e + 32, cols].astype(BF16).T

        def prep_jobs(j, e):
            def kb_job(beta, d):
                r = Dh * e + d
                w = min(128, 8 * NG - 128 * beta)
                val = jnp.broadcast_to(kv_s[j, r:r + 1, beta * 128:beta * 128 + w], (128, w)).T

                def put(i):
                    y_s[e][zero + (KB0 + (16 * beta + i) * Dh + d)] = val[8 * i:8 * i + 8]
                    return [val[8 * i:8 * i + 8]]
                return [functools.partial(put, i) for i in range(min(16, NG - 16 * beta))]

            def kw_job(c):
                kw = pltpu.bitcast(k_window(j, e, slice(c * 128, (c + 1) * 128)), F32)

                def put(t):
                    y_s[e][zero + (KW0 + 8 * c + t), :, 0:32] = kw[8 * t:8 * t + 8]
                    return []
                return [functools.partial(put, t) for t in range(-(-(128 - 8 * G[c]) // 16))]
            a = [functools.partial(kb_job, beta, d) for beta in range(NVB) for d in range(Dh)]
            b = [functools.partial(kw_job, c) for c in range(NC)]
            return [job for x, y in zip(_spread(a, NC), b) for job in [y] + x]

        def whole(job):
            return lambda: [v for put in job() for v in put()]

        for l in range(NL):
            cp_x[l].start()
            cp_x[NL + l].start()
            if delay and l < NL - 1:
                pl.delay(delay)
        cp_w[0].start()
        later = []
        for l in range(NL):
            for c in ([], [cp_w[1]], [], cp_w[2:])[l]:
                c.start()
            mark("x%d" % l, lambda: (cp_x[l].wait(), cp_x[NL + l].wait()))
            if 1 in phases:
                jobs = norm_jobs(strassen[0], 0, l, 0, True)
                for job in jobs[:2 * NB] + later:
                    job()
                later = jobs[2 * NB:]
        for c in cp_x[2 * NL:]:
            c.start()
        if scopes:
            with jax.named_scope("ln0_done"):
                cp_w[1].wait()
        else:
            cp_w[1].wait()
        cp_w[0].wait()
        for job in (qkv_jobs[0] if 1 in phases else []) + later:
            job()

        def dma_job(waits, starts):
            for c in starts:
                c.start()
            if scopes:
                with jax.named_scope("dma_wait_%d" % len(waits)):
                    for c in waits:
                        c.wait()
            else:
                for c in waits:
                    c.wait()
            return []
        for t in range(NT):
            side = [[] for _ in range(3 * NB)]
            if t == 0:
                for r in range(3 * NB - 1):
                    side[r] += qkv_jobs[r + 1]
            if t + 1 < NT:
                nxt = [job for l in range(NL) for job in norm_jobs(strassen[0], t + 1, l, (t + 1) % 2, True)]
                for r, jobs in enumerate(_spread(nxt, 3 * NB - ln_at)):
                    side[ln_at + r] = [x for p in zip(_spread(side[ln_at + r], 3), _spread(jobs, 3)) for q in p for x in q]
            else:
                for r, jobs in enumerate(_spread(tail_jobs, 2 * NB + 1)):
                    side[r] += jobs
                last = [functools.partial(gather_job, i) for i in range(D // 8)]
                last = last[:8] + [x for p in zip(_spread(last[8:], 8), _spread([whole(job) for job in prep_jobs(zero, 0)], 8)) for q in p for x in q]
                for r, jobs in enumerate(_spread(last, NB - 1)):
                    side[2 * NB + 1 + r] += jobs
            for r in range(3 * NB):
                if t == 0 and r == ln_at:
                    side[r] = [lambda: []] + [functools.partial(dma_job, cp_w[2:] + cp_x[2 * NL:], [cp_wo, cp_w1, cp_w2])] + side[r]
                if t == NT - 1 and r == 0:
                    side[r] = [lambda: []] * 4 + [functools.partial(dma_job, [cp_wo, cp_w1, cp_w2], [])] + side[r]
                if 1 not in phases:
                    for job in side[r]:
                        if getattr(job, "func", None) is dma_job:
                            job()
                if 1 not in phases:
                    continue
                c = block_product(strassen[0], *weight_operands(aq_s[r % 2], 16 * (r // 2), 64, KH), *get_right(t % 2), jobs=side[r])
                dst = (qt_s, kt_s, vt_s)[r // NB]
                for i in range(2):
                    for k in range(2):
                        v = c[i][k] * (Dh ** -0.5 * LOG2E) if r < NB else c[i][k]
                        rows_put(dst, 128 * (r % NB) + 64 * i, v.astype(BF16).astype(F32), slice(t * TB + k * TQ, t * TB + (k + 1) * TQ))

        subq = lax.broadcasted_iota(jnp.int32, (8, TQ), 0)
        row32 = lax.broadcasted_iota(jnp.int32, (32, TQ), 0)

        def q_window(j, e, cols):
            qw = qt_s[j, 8 * e:8 * e + 32, cols]
            return jnp.where(row32 < Dh if e == 0 else row32 >= 32 - Dh, qw, 0.0).astype(BF16)

        def v_pieces(j, e, cols):
            if e == 0:
                return [vt_s[j, 0:8, cols], vt_s[j, 8:16, cols], jnp.where(sub < 4, vt_s[j, 16:24, cols], 1.0)]
            return [jnp.where(sub >= 4, vt_s[j, 16:24, cols], 1.0), vt_s[j, 24:32, cols], vt_s[j, 32:40, cols]]

        def fast_pair(j, bad, first_only=False):
            jn = jnp.minimum(j + 1, NP - 1)
            items = [(e, qb, c) for e in range(2) for qb in range(NQ) for c in range(NC)]
            prep = []
            for (pj, pe) in ((j, 1), (jn, 0)):
                prep += _spread(prep_jobs(pj, pe), NQ * NC - pad) + [[] for _ in range(pad)]
            vres, accs = {}, {}
            state = {"bad": bad, "puts": []}

            def run(job):
                n, us, l, d0, d1 = job
                e, qb, c = items[n % len(items)]
                jq = j if n < len(items) else jn
                for u in us:
                    acc = vres.get((n, u, l))
                    for d in range(d0, d1):
                        r = Dh * e + d
                        q = jnp.broadcast_to(qt_s[jq, r:r + 1, qb * TQ + l * 128:qb * TQ + (l + 1) * 128], (8, 128))
                        t = y_s[e][KB0 + (goff[c] + u) * Dh + d] * q
                        acc = t if acc is None else acc + t
                    vres[(n, u, l)] = jnp.exp2(acc) if d1 == Dh else acc
                return [(n, u, l) for u in us]

            def todo(n):
                g = G[n % NC]
                cuts = [(Dh * i) // seg for i in range(seg + 1)]
                return [(n, (u, u + 1), l, cuts[i], cuts[i + 1]) for u in range(0, g, 2) for l in range(NL) for i in range(seg)]

            flat = [job for n in range(len(items) + NC) for job in todo(n)]
            per_loop = sum(len(todo(n)) for n in range(len(items)))
            slots = _spread(flat[lead:lead + per_loop], sum(8 - G[c] // 2 for _, _, c in items))
            where = {}
            for job in flat:
                for u in job[1]:
                    where.setdefault((job[0], u, job[2]), PV0 + len(where) % NPV)

            def tie(load, jobs, e):
                for job in jobs:
                    for key in run(job):
                        y_s[e][where[key]] = vres[key]
                return load()

            def do_pv(n, p):
                e, qb, c = items[n]
                vt = jnp.concatenate(v_pieces(j, e, slice(c * 128, (c + 1) * 128)), axis=0)
                pv = jnp.dot(vt, p, preferred_element_type=F32)
                busy = bool(prep[n] or state["puts"])
                for put in state["puts"]:
                    put()
                state["puts"] = []
                for job in prep[n]:
                    puts = job()
                    for put in puts[:early]:
                        put()
                    state["puts"] += puts[early:]
                if c == 0:
                    acc = pv
                else:
                    acc = accs[(e, qb)]
                    if busy:
                        a0 = jnp.concatenate([y_s[1 - e][zero + AC0], acc[0:8, 128:]], axis=1)
                        acc = jnp.concatenate([a0, acc[8:]], axis=0)
                    acc = acc + pv
                accs[(e, qb)] = acc
                if n + 1 < len(items) and (prep[n + 1] or state["puts"]):
                    y_s[1 - e][AC0] = acc[0:8, 0:128]
                if c == NC - 1:
                    cols = slice(qb * TQ, (qb + 1) * TQ)
                    l = acc[23:24] if e == 0 else acc[0:1]
                    good = (l >= L_MIN) & (l <= L_MAX)
                    amax = jnp.maximum(jnp.maximum(jnp.abs(acc[0:8]), jnp.abs(acc[8:16])), jnp.abs(acc[16:24]))
                    state["bad"] = jnp.where(good & (amax <= O_MAX), state["bad"], 1.0)
                    o = acc * (1.0 / l)
                    if e == 0:
                        ot_s[j, 0:24, cols] = o
                    else:
                        ot_s[j, 16:24, cols] = jnp.where(subq < 4, ot_s[j, 16:24, cols], o[0:8])
                        ot_s[j, 24:40, cols] = o[8:24]

            if first_only:
                for job in flat[:lead]:
                    for (n, u, l) in run(job):
                        y_s[1][where[(n + len(items), u, l)]] = vres[(n, u, l)]
                return
            for job in flat[:lead]:
                for u in job[1]:
                    vres[(job[0], u, job[2])] = y_s[1][where[(job[0] + len(items), u, job[2])]]
            pend = None
            slots = iter(slots)
            for n, (e, qb, c) in enumerate(items):
                if c == 0:
                    qw = q_window(j, e, slice(qb * TQ, (qb + 1) * TQ))
                g = G[c]
                npc = 8 - g // 2
                pieces = [tie(lambda: y_s[e][zero + (KW0 + c * 8 + npc - 1 - t), :, 0:32], next(slots), e) for t in range(npc)]
                r = jnp.dot(_as_bf16(jnp.concatenate(pieces, axis=0)), qw, preferred_element_type=F32)
                pm = jnp.exp2(jnp.concatenate([r[16 * (npc - 1 - t):16 * (npc - t)] for t in range(npc)], axis=0))
                pvv = [jnp.concatenate([vres[(n, u, l)] for l in range(NL)], axis=1) for u in range(g)]
                p = jnp.concatenate([pm] + pvv, axis=0)
                if pend is not None:
                    do_pv(*pend)
                pend = (n, p)
            do_pv(*pend)
            return state["bad"]

        def safe_pair(t, carry):
            j, qb = t // NQ, t % NQ
            cols = pl.ds(pl.multiple_of(qb * TQ, TQ), TQ)
            outs = []
            for e in range(2):
                qw = q_window(j, e, cols)

                def scores(c):
                    return jnp.dot(k_window(j, e, pl.ds(pl.multiple_of(c * 128, 128), 128)), qw, preferred_element_type=F32)

                def max_body(c, m):
                    return jnp.maximum(m, jnp.max(scores(c), axis=0, keepdims=True))
                m = lax.fori_loop(0, NC, max_body, jnp.full((1, TQ), -jnp.inf, F32))

                def pv_body(c, acc):
                    p = jnp.exp2(scores(c) - m).astype(BF16)
                    vt = jnp.concatenate(v_pieces(j, e, pl.ds(pl.multiple_of(c * 128, 128), 128)), axis=0)
                    return acc + jnp.dot(vt, p, preferred_element_type=F32)
                acc = lax.fori_loop(0, NC, pv_body, jnp.zeros((24, TQ), F32))
                outs.append(acc * (1.0 / (acc[23:24] if e == 0 else acc[0:1])))
            mid = jnp.where(subq < 4, outs[0][16:24], outs[1][0:8])
            ot_s[j, :, cols] = jnp.concatenate([outs[0][0:16], mid, outs[1][8:24]], axis=0)
            return carry

        if 2 in phases:
            fast_pair(zero, None, True)
            if scopes:
                with jax.named_scope("attn"):
                    bad = lax.fori_loop(0, NP, fast_pair, jnp.zeros((8, TQ), F32))
            else:
                bad = lax.fori_loop(0, NP, fast_pair, jnp.zeros((8, TQ), F32))
            if fallback:
                @pl.when(jnp.max(bad) > 0.0)
                def _():
                    lax.fori_loop(0, NP * NQ, safe_pair, 0)

        def bias_rows(r0, n):
            return jnp.concatenate([bias_s[r0:r0 + n, :]] * NL, axis=1)

        def tiles(t, k):
            return range(k * NL, (k + 1) * NL)

        def attn_jobs(t):
            def rows(l, k, r0, n):
                tok = t * TB + k * TQ + l * 128
                return rows_get(ot_s, r0, n, slice(tok, tok + 128))
            per_tile = [right_jobs(strassen[1], 2 + t % 2, l, functools.partial(rows, l)) for l in range(NL)]
            return [job for group in zip(*per_tile) for job in group]

        def out_proj(t, jobs):
            jobs = _spread(jobs, NB)
            for r in range(NB):
                c = block_product(strassen[1], *weight_operands(a_s, A_O + 16 * r, 64, KH), *get_right(2 + t % 2), jobs=jobs[r])
                for i in range(2):
                    rr = slice(128 * r + 64 * i, 128 * r + 64 * i + 64)
                    for k in range(2):
                        for l, tile in enumerate(tiles(t, k)):
                            xt_s[t][tile, rr] = xt_s[t][tile, rr] + c[i][k][:, 128 * l:128 * l + 128]

        def act_jobs(t, r, c):
            def job(r0, n):
                act = []
                for u in range(4):
                    g = jnp.maximum(c[u // 2][u % 2][r0:r0 + n] + bias_rows(2 * R1 * r + R1 * (u // 2) + r0, n), 0.0)
                    act.append(g * g)
                out = []
                for i in range(7 if strassen[3] else 4):
                    v = _as_u32(right_operand(strassen[3], i, lambda u: act[u]))
                    c_s[t % 2][i, (R1 * r + r0) // 2:(R1 * r + r0 + n) // 2, :] = v
                    out += groups(v)
                return out
            return [functools.partial(job, r0, 16) for r0 in range(0, R1, 16)]

        def ffn_up(t, jobs, carried):
            jobs = _spread(jobs, NF)
            for r in range(NF):
                side = [x for p in zip(_spread(carried, 7), _spread(jobs[r], 7)) for q in p for x in q]
                c = block_product(strassen[2], *weight_operands(a_s, A_1 + 16 * r, R1, KH), *get_right(t % 2), jobs=side)
                carried = act_jobs(t, r, c)
                if not defer:
                    for job in carried:
                        job()
                    carried = []
            return carried

        def ffn_down(t, pending, carried=()):
            for r in range(NB):
                a, _ = weight_operands(a_s, A_2 + 7 * (F // 256) * r, 64, F // 2)
                c = block_product(strassen[3], a, None, lambda i: _as_bf16(c_s[t % 2][i]), None, jobs=carried if r == 0 else ())
                for cp in pending:
                    cp.start()
                rr = slice(128 * r, 128 * r + 128)
                for k in range(2):
                    y = jnp.concatenate([c[0][k], c[1][k]], axis=0) + bias_rows(F + 128 * r, 128)
                    for l, tile in enumerate(tiles(t, k)):
                        o_v[zero + (t * NB + r), tile * 128:(tile + 1) * 128, :] = (xt_s[t][tile, rr] + y[:, 128 * l:128 * l + 128]).astype(BF16).T
                pending = [cp_o[t][r]]
            return pending

        if 3 in phases:
            ln2 = lambda t: [job for l in range(NL) for job in norm_jobs(strassen[2], t, l, t % 2, False)]
            for job in attn_jobs(0):
                job()
            out_proj(0, attn_jobs(1))
            out_proj(1, ln2(0))
            carried = ffn_up(1, [], ffn_up(0, ln2(1), []))
            for cp in ffn_down(1, ffn_down(0, [], carried)):
                cp.start()
        else:
            for t in range(NT):
                for r in range(NB):
                    cp_o[t][r].start()
        if scopes:
            with jax.named_scope("out_wait"):
                cp_o[0][0].wait()
        else:
            cp_o[0][0].wait()
        for t in range(NT):
            for r in range(NB):
                if t or r:
                    cp_o[t][r].wait()

    n_a = 16 * NB + 16 * (F // (2 * R1)) + 7 * NB * (F // 256)

    @jax.jit
    def run(A_x, A_wqkv, A_wo, B_x, B_w1, B_b1, B_w2, B_b2):
        del B_x
        anyspec = pl.BlockSpec(memory_space=pl.ANY)
        vmem = pl.BlockSpec(memory_space=pltpu.VMEM)
        return pl.pallas_call(
            kernel,
            out_shape=jax.ShapeDtypeStruct((1, S, D), BF16),
            in_specs=[pl.BlockSpec(memory_space=pltpu.SMEM), anyspec, anyspec, anyspec, anyspec, vmem, anyspec, vmem],
            out_specs=anyspec,
            scratch_shapes=[
                pltpu.VMEM((S, D), BF16), pltpu.VMEM((D, 3 * D), BF16), pltpu.VMEM((D, D), BF16),
                pltpu.VMEM((D, F), BF16), pltpu.VMEM((F, D), BF16), pltpu.VMEM((NT * NB, TB, 128), BF16),
                [pltpu.VMEM((2 * NL, D, 128), F32)] * NT,
                pltpu.VMEM((NP, 2 * Dh, S), F32), pltpu.VMEM((NP, 2 * Dh, S), F32),
                pltpu.VMEM((NP, 2 * Dh, S), F32), pltpu.VMEM((NP, 2 * Dh, S), F32),
                pltpu.VMEM((NP, 2 * Dh, NVB * 128), F32),
                [pltpu.VMEM((NY, 8, 128), F32)] * 2,
                [pltpu.VMEM((16 * 8, 32, 128), U32)] * 2,
                pltpu.VMEM((n_a, R1 // 2, 128), U32),
                [pltpu.VMEM((8, KH // 2, TQ), U32)] * 4,
                [pltpu.VMEM((7, F // 4, TQ), U32)] * 2,
                pltpu.VMEM((F + D, 128), F32),
                pltpu.SemaphoreType.DMA((2 * NL + 1,)), pltpu.SemaphoreType.DMA((len(w_cuts) - 1,)),
                pltpu.SemaphoreType.DMA((3 + NT * NB,)),
            ],
            compiler_params=pltpu.CompilerParams(vmem_limit_bytes=110 * 2**20, flags=flags),
        )(jnp.zeros((1,), jnp.int32), A_x, A_wqkv, A_wo, B_w1, B_b1, B_w2, B_b2)
    return run


_run = make(lead=8)


def pallas_sequential_preLN__softmax_full_mha__dense_activation_squared_relu__prompt_kernel(A_x, A_wqkv, A_wo, B_x, B_w1, B_b1, B_w2, B_b2):
    return _run(A_x, A_wqkv, A_wo, B_x, B_w1, B_b1, B_w2, B_b2)
```

```python
import functools

import jax
import jax.experimental.pallas as pl
import jax.experimental.pallas.tpu as pltpu
import jax.numpy as jnp
from jax import lax

F32, BF16, U32 = jnp.float32, jnp.bfloat16, jnp.uint32
HEADS = 32
EPS = 1e-5
LOG2E = 1.4426950408889634
L_MIN, L_MAX, O_MAX = 2.0 ** -60, 2.0 ** 100, 2.0 ** 120

TQ = 512
TB = 2 * TQ
NL = TQ // 128
R = 64
RP = 16
VG = 2
SEG = 4
PAD = 4
W_CUTS = (0, 2, 7, 15)
LN_AT = 6


def _as_bf16(x):
    return pltpu.bitcast(x, BF16)


def _as_u32(x):
    return pltpu.bitcast(x, U32)


def _spread(jobs, n):
    cut = [(i * len(jobs)) // n for i in range(n + 1)]
    return [jobs[cut[i]:cut[i + 1]] for i in range(n)]


def _spread_cost(jobs, n):
    total, seen, out = sum(c for _, c in jobs), 0, [[] for _ in range(n)]
    for job, c in jobs:
        out[min(n - 1, (2 * seen + c) * n // (2 * total))].append(job)
        seen += c
    return out


def _interleave(a, b):
    return [job for pair in zip(a, b) for part in pair for job in part]


def _nothing():
    return []


def _registers(v):
    return [v[8 * i:8 * i + 8, 128 * k:128 * k + 128] for k in range(v.shape[1] // 128) for i in range(v.shape[0] // 8)]


def _left_operand(i, blk):
    f = lambda u: blk(u).astype(F32)
    return (lambda: (f(0) + f(3)).astype(BF16), lambda: (f(2) + f(3)).astype(BF16), lambda: blk(0), lambda: blk(3),
            lambda: (f(0) + f(1)).astype(BF16), lambda: (f(2) - f(0)).astype(BF16), lambda: (f(1) - f(3)).astype(BF16))[i]()


def _right_operand(i, blk):
    return (lambda: blk(0) + blk(3), lambda: blk(0), lambda: blk(1) - blk(3), lambda: blk(2) - blk(0),
            lambda: blk(3), lambda: blk(0) + blk(1), lambda: blk(2) + blk(3))[i]().astype(BF16)


def _kernel(z_ref, x_hbm, wqkv_hbm, wo_hbm, w1_hbm, b1_ref, w2_hbm, b2_ref, o_hbm,
            x_v, wqkv_v, wo_v, w1_v, w2_v, o_v, xt_s, qt_s, kt_s, vt_s, ot_s, kv_s, y_s, aq_s, a_s, b_s, c_s,
            bias_s, chk_s, acc_s, sem_x, sem_w, sems):
    S, D = x_v.shape
    F = w1_v.shape[1]
    Dh = D // HEADS
    NP, NB, NC, NQ, NT, NF = HEADS // 2, D // 128, S // 128, S // TQ, S // TB, F // (2 * R)
    KH = (D // 256) * 128
    NG = VG * NC
    KB0, KW0 = 0, NG * Dh
    PV0 = KW0 + NC * 8
    AC0 = y_s[0].shape[0] - 1
    A_O, A_1 = 0, 16 * NB
    A_2 = A_1 + 16 * NF

    zero = z_ref[0]
    sub = lax.broadcasted_iota(jnp.int32, (8, 128), 0)
    lane = lax.broadcasted_iota(jnp.int32, (8, 128), 1)
    always = (sub + zero) >= 0
    products = []

    x_cuts = [128 * i for i in range(2 * NL + 1)] + [S]
    cp_x = [pltpu.make_async_copy(x_hbm.at[0, pl.ds(a, b - a)], x_v.at[pl.ds(a, b - a)], sem_x.at[i])
            for i, (a, b) in enumerate(zip(x_cuts, x_cuts[1:]))]
    cp_w = [pltpu.make_async_copy(wqkv_hbm.at[:, pl.ds(128 * a, 128 * (b - a))], wqkv_v.at[:, pl.ds(128 * a, 128 * (b - a))], sem_w.at[i])
            for i, (a, b) in enumerate(zip(W_CUTS, W_CUTS[1:]))]
    cp_tail = [pltpu.make_async_copy(src, dst, sems.at[i]) for i, (src, dst) in enumerate(((wo_hbm, wo_v), (w1_hbm, w1_v), (w2_hbm, w2_v)))]
    cp_o = [[pltpu.make_async_copy(o_v.at[t * NB + r], o_hbm.at[0, pl.ds(t * TB, TB), pl.ds(r * 128, 128)], sems.at[3 + t * NB + r])
             for r in range(NB)] for t in range(NT)]

    def rows_get(ref, r0, n, cols):
        return jnp.concatenate([ref[i // 5, 8 * (i % 5):8 * (i % 5) + 8, cols] for i in range(r0 // 8, (r0 + n) // 8)], axis=0)

    def rows_put(ref, r0, val, cols):
        for k in range(val.shape[0] // 8):
            i = r0 // 8 + k
            ref[i // 5, 8 * (i % 5):8 * (i % 5) + 8, cols] = val[8 * k:8 * k + 8]

    def after(val, jobs):
        deps = [pltpu.bitcast(v, val.dtype) for job in jobs for v in job()]
        if not deps:
            return val
        nr = val.shape[0] // 8
        tiles = _registers(val)
        for i, vs in enumerate(_spread(deps, len(tiles))[::-1]):
            for v in vs:
                tiles[i] = jnp.where(always, tiles[i], v)
        return jnp.concatenate([jnp.concatenate(tiles[i::nr], axis=1) for i in range(nr)], axis=0)

    def block_product(a, ar, b, br, jobs, half_done=None):
        js = iter(_spread(list(jobs), 7 if ar is None else 11))

        def mm(l, r):
            v = jnp.dot(l, r, preferred_element_type=F32)
            out = after(v, next(js))
            products.append(v[0:8, 0:128])
            return out
        rest = (lambda c, i, k: c) if ar is None else (lambda c, i, k: c + mm(ar(i), br(k)))
        m = lambda i: mm(a(i), b(i))
        m1 = m(0)
        m4 = m(3)
        m5 = m(4)
        c11 = rest(m1 + m4 - m5 + m(6), 0, 0)
        m2 = m(1)
        c21 = rest(m2 + m4, 1, 0)
        if half_done is not None:
            left = list(js)
            js = iter([x + y for x, y in zip(left, _spread(half_done(c11, c21), len(left)))])
        m3 = m(2)
        c12 = rest(m3 + m5, 0, 1)
        c22 = rest(m1 - m2 + m3 + m(5), 1, 1)
        return [[c11, c12], [c21, c22]]

    def weight_jobs(a_ref, base, kh, nrest, load):
        nk = kh // 128
        memo = []

        def blk(u):
            if not memo:
                wt = load().T
                memo.extend((wt[0:R], wt[R:2 * R]))
            return memo[u // 2][:, (u % 2) * kh:(u % 2 + 1) * kh]

        def main(i):
            v = _as_u32(_left_operand(i, blk))
            for k in range(nk):
                a_ref[zero + (base + i * nk + k), 0:R // 2] = v[:, 128 * k:128 * k + 128]
            return _registers(v)

        def rest(i):
            blk(0)
            v = _as_u32(memo[i][:, 2 * kh:])
            a_ref[zero + (base + 7 * nk + i), 0:R // 2] = v
            return _registers(v)
        return [functools.partial(main, i) for i in range(7)] + [functools.partial(rest, i) for i in range(nrest)]

    def weight_operands(a_ref, base, kh):
        nk = kh // 128
        a = lambda i: _as_bf16(jnp.concatenate([a_ref[base + i * nk + k, 0:R // 2] for k in range(nk)], axis=1))
        return a, (lambda i: _as_bf16(a_ref[base + 7 * nk + i, 0:R // 2]))

    def right_jobs(slot, l, rows):
        def main(r0):
            blk = [rows(u % 2, (u // 2) * KH + r0, RP) for u in range(4)]
            out = []
            for i in range(7):
                v = _as_u32(_right_operand(i, lambda u: blk[u]))
                b_s[slot][zero + i, r0 // 2:(r0 + RP) // 2, 128 * l:128 * l + 128] = v
                out += _registers(v)
            return out

        def rest(k):
            v = _as_u32(rows(k, 2 * KH, D - 2 * KH).astype(BF16))
            b_s[slot][zero + 7, 64 * k:64 * k + 64, 128 * l:128 * l + 128] = v
            return _registers(v)
        return [(functools.partial(main, r0), 7) for r0 in range(0, KH, RP)] + [(functools.partial(rest, k), 7) for k in range(2)]

    def right_operands(slot):
        return (lambda i: _as_bf16(b_s[slot][i])), (lambda k: _as_bf16(b_s[slot][7, 64 * k:64 * k + 64]))

    def norm_jobs(t, l, from_x):
        tile = [k * NL + l for k in range(2)]
        mean, rstd, part = {}, {}, {}

        def add_up(key, v):
            v = [v[8 * i:8 * i + 8] for i in range(v.shape[0] // 8)] + ([part[key]] if key in part else [])
            while len(v) > 1:
                v = [v[i] + v[i + 1] for i in range(0, len(v) - 1, 2)] + v[len(v) - len(v) % 2:]
            part[key] = v[0]
            return v

        def mean_job(k, b):
            rr = slice(128 * b, 128 * b + 128)
            if from_x:
                v = x_v[t * TB + tile[k] * 128:t * TB + (tile[k] + 1) * 128, rr].T.astype(F32)
                xt_s[t][zero + tile[k], rr] = v
            else:
                v = after(xt_s[t][tile[k], rr], [lambda: products[-1:]])
            out = add_up(("sum", k), v)
            if b == NB - 1:
                mean[k] = jnp.broadcast_to(jnp.sum(out[0], axis=0, keepdims=True) * (1.0 / D), (8, 128))
                out = [mean[k]]
            return out

        def centered(k, r0, n):
            return (xt_s[t][zero + tile[k], r0:r0 + n].reshape(n // 8, 8, 128) - mean[k][None]).reshape(n, 128)

        def var_job(k, b):
            d = centered(k, 128 * b, 128)
            out = add_up(("var", k), d * d)
            if b == NB - 1:
                rstd[k] = jnp.broadcast_to(lax.rsqrt(jnp.sum(out[0], axis=0, keepdims=True) * (1.0 / D) + EPS), (8, 128))
                out = [rstd[k]]
            return out

        def rows(k, r0, n):
            return (centered(k, r0, n).reshape(n // 8, 8, 128) * rstd[k][None]).reshape(n, 128)
        costs = ((mean_job, 8 if from_x else 2), (var_job, 5))
        return [(functools.partial(job, k, b), cost) for job, cost in costs for k in range(2) for b in range(NB)] + right_jobs(t % 2, l, rows)

    def norm_block(t, from_x):
        per_tile = [norm_jobs(t, l, from_x) for l in range(NL)]
        passes = lambda l, i: (per_tile[l][:2 * NB], per_tile[l][2 * NB:4 * NB], per_tile[l][4 * NB:])[i] if 0 <= l < NL else []
        return [job for step in range(NL + 2) for group in zip(*[_spread(passes(step - i, i), 2 * NB) for i in range(3)])
                for jobs in group for job in jobs]

    def w2_columns(r):
        w = w2_v[:, 128 * r:128 * r + 128]
        return jnp.concatenate([w[2 * R * q + R * i:2 * R * q + R * (i + 1)] for i in range(2) for q in range(NF)], axis=0)

    def bias_job(ref, base, r):
        bias = ref[...].astype(F32).reshape(1, ref.shape[0])
        v = jnp.broadcast_to(bias[:, 128 * r:128 * r + 128], (128, 128)).T
        bias_s[base + 128 * r:base + 128 * r + 128, :] = v
        return _registers(v)

    columns = lambda ref, r: lambda: ref[:, 128 * r:128 * r + 128]
    qkv_jobs = [weight_jobs(aq_s[r % 2], 16 * (r // 2), KH, 2, columns(wqkv_v, r)) for r in range(3 * NB)]
    tail_jobs = [job for r in range(NB) for job in weight_jobs(a_s, A_O + 16 * r, KH, 2, columns(wo_v, r))]
    tail_jobs += [job for r in range(NF) for job in weight_jobs(a_s, A_1 + 16 * r, KH, 2, columns(w1_v, r))]
    tail_jobs += [job for r in range(NB) for job in weight_jobs(a_s, A_2 + 7 * (F // 256) * r, F // 2, 0, functools.partial(w2_columns, r))]
    tail_jobs += [functools.partial(bias_job, ref, base, r) for ref, base in ((b1_ref, 0), (b2_ref, F)) for r in range(ref.shape[0] // 128)]

    def gather_job(i):
        p, rr = i // 5, slice(8 * (i % 5), 8 * (i % 5) + 8)
        out = []
        for beta in range(NG // 16):
            acc = jnp.zeros((8, 128), F32)
            for k in range(16 // VG):
                c, lo = beta * (16 // VG) + k, 8 * VG * k
                v = kt_s[zero + p, rr, 128 * c:128 * c + 128]
                shift = (lo + 8 * VG) % 128
                v = pltpu.roll(v, shift, 1) if shift else v
                acc = jnp.where((lane >= lo) & (lane < lo + 8 * VG), v, acc)
            kv_s[p, rr, 128 * beta:128 * beta + 128] = acc
            out.append(acc)
        return out

    def k_window(j, e, cols):
        return kt_s[j, 8 * e:8 * e + 32, cols].astype(BF16).T

    def prep_jobs(j, e):
        def kb_job(beta, d):
            r = Dh * e + d
            val = jnp.broadcast_to(kv_s[j, r:r + 1, beta * 128:beta * 128 + 128], (128, 128)).T

            def put(i):
                y_s[e][zero + (KB0 + (16 * beta + i) * Dh + d)] = val[8 * i:8 * i + 8]
                return [val[8 * i:8 * i + 8]]
            return [functools.partial(put, i) for i in range(16)]

        def kw_job(c):
            kw = pltpu.bitcast(k_window(j, e, slice(c * 128, (c + 1) * 128)), F32)

            def put(t):
                y_s[e][zero + (KW0 + 8 * c + t), :, 0:32] = kw[8 * t:8 * t + 8]
                return []
            return [functools.partial(put, t) for t in range(8 - VG // 2)]
        a = [functools.partial(kb_job, beta, d) for beta in range(NG // 16) for d in range(Dh)]
        return [job for c, x in enumerate(_spread(a, NC)) for job in [functools.partial(kw_job, c)] + x]

    for l in range(NL):
        cp_x[l].start()
        cp_x[NL + l].start()
    cp_w[0].start()
    later = []
    for l in range(NL):
        for c in ([], [cp_w[1]], [], [cp_w[2]])[l]:
            c.start()
        cp_x[l].wait()
        cp_x[NL + l].wait()
        jobs = [job for job, _ in norm_jobs(0, l, True)]
        for job in jobs[:2 * NB] + later:
            job()
        later = jobs[2 * NB:]
    cp_x[2 * NL].start()
    cp_w[0].wait()
    for job in qkv_jobs[0] + later:
        job()

    def dma_job(waits, starts):
        for c in starts:
            c.start()
        for c in waits:
            c.wait()
        return []

    def qkv_store(t, r, i, k, v):
        if r < NB:
            v = v * (Dh ** -0.5 * LOG2E)
        elif r >= 2 * NB:
            v = v.astype(BF16).astype(F32)
        rows_put((qt_s, kt_s, vt_s)[r // NB], 128 * (r % NB) + R * i, v, slice(t * TB + k * TQ, t * TB + (k + 1) * TQ))
        return _registers(v)

    side = [qkv_jobs[1:] + [[]], _spread(tail_jobs, 3 * NB)]
    for r, jobs in enumerate(_spread_cost(norm_block(1, True), 3 * NB - LN_AT - 1)):
        side[0][LN_AT + r] = _interleave(_spread(side[0][LN_AT + r], 3), _spread(jobs, 3))
    last = [functools.partial(gather_job, i) for i in range(D // 8)]
    first_head = [lambda job=job: [v for put in job() for v in put()] for job in prep_jobs(zero, 0)]
    for r, jobs in enumerate(_spread(last[:8] + _interleave(_spread(last[8:], 8), _spread(first_head, 8)), 2 * NB - 1)):
        side[1][NB + 1 + r] = side[1][NB + 1 + r] + jobs
    dmas = {(0, W_CUTS[1] - 1): [_nothing] * 2 + [functools.partial(dma_job, [cp_w[1]], [])],
            (0, LN_AT): [_nothing, functools.partial(dma_job, [cp_w[2], cp_x[2 * NL]], cp_tail)],
            (1, 0): [_nothing] * 4 + [functools.partial(dma_job, cp_tail, [])]}
    orders = (range(3 * NB), [*range(NB, 2 * NB), *range(NB), *range(2 * NB, 3 * NB)])
    carried = []
    for t in range(NT):
        for step, r in enumerate(orders[t]):
            jobs = dmas.get((t, step), []) + _interleave(_spread(carried, 4), _spread(side[t][step], 4))
            c = block_product(*weight_operands(aq_s[r % 2], 16 * (r // 2) + (0 if t else zero), KH), *right_operands(t % 2), jobs)
            carried = [functools.partial(qkv_store, t, r, i, k, c[i][k]) for k in range(2) for i in range(2)]
    for job in carried:
        job()

    subq = lax.broadcasted_iota(jnp.int32, (8, TQ), 0)
    row32 = lax.broadcasted_iota(jnp.int32, (32, TQ), 0)

    def q_window(j, e, cols):
        qw = qt_s[j, 8 * e:8 * e + 32, cols]
        return jnp.where(row32 < Dh if e == 0 else row32 >= 32 - Dh, qw, 0.0).astype(BF16)

    def v_window(j, e, cols):
        if e == 0:
            pieces = [vt_s[j, 0:8, cols], vt_s[j, 8:16, cols], jnp.where(sub < 4, vt_s[j, 16:24, cols], 1.0)]
        else:
            pieces = [jnp.where(sub >= 4, vt_s[j, 16:24, cols], 1.0), vt_s[j, 24:32, cols], vt_s[j, 32:40, cols]]
        return jnp.concatenate(pieces, axis=0)

    def finish(j, e, qb, acc):
        cols = slice(qb * TQ, (qb + 1) * TQ)
        inv = 1.0 / (acc[23:24] if e == 0 else acc[0:1])
        o = acc * inv
        inv8 = jnp.broadcast_to(inv, (8, TQ))
        for i, (f, v) in enumerate(((jnp.maximum, inv8), (jnp.minimum, inv8), (jnp.add, o))):
            chk_s[i, j, e * NQ + qb] = functools.reduce(f, _registers(v))
        if e == 0:
            ot_s[j, 0:Dh, cols] = o[0:Dh]
        else:
            ot_s[j, Dh:24, cols] = o[4:8]
            ot_s[j, 24:40, cols] = o[8:24]

    def unshifted_pair(j, carry):
        jn = jnp.minimum(j + 1, NP - 1)
        items = [(e, qb, c) for e in range(2) for qb in range(NQ) for c in range(NC)]
        prep = []
        for pj, pe in ((j, 1), (jn, 0)):
            prep += _spread(prep_jobs(pj, pe), NQ * NC - PAD) + [[] for _ in range(PAD)]
        scores, accs, puts, slot = {}, {}, [], {}
        npc = 8 - VG // 2
        cuts = [(Dh * i) // SEG for i in range(SEG + 1)]
        work = iter(_spread([(n, l, cuts[i], cuts[i + 1]) for n in range(len(items)) for l in range(NL) for i in range(SEG)], npc * len(items)))

        def key_piece(e, c, t):
            for n, l, d0, d1 in next(work):
                ne, nqb, nc = items[n]
                for g in range(VG):
                    acc = scores.get((n, g, l))
                    for d in range(d0, d1):
                        r = Dh * ne + d
                        q = jnp.broadcast_to(qt_s[j, r:r + 1, nqb * TQ + l * 128:nqb * TQ + (l + 1) * 128], (8, 128))
                        term = y_s[ne][KB0 + (VG * nc + g) * Dh + d] * q
                        acc = term if acc is None else acc + term
                    scores[(n, g, l)] = jnp.exp2(acc) if d1 == Dh else acc
                for g in range(VG):
                    y_s[e][slot.setdefault((n, g, l), PV0 + len(slot) % (AC0 - PV0))] = scores[(n, g, l)]
            return y_s[e][zero + (KW0 + c * 8 + t), :, 0:32]

        def accumulate(n, p):
            e, qb, c = items[n]
            pv = jnp.dot(v_window(j, e, slice(c * 128, (c + 1) * 128)), p, preferred_element_type=F32)
            busy = bool(prep[n] or puts)
            while puts:
                puts.pop(0)()
            for job in prep[n]:
                todo = job()
                todo.pop(0)()
                puts.extend(todo)
            if c == 0:
                acc = pv
            else:
                acc = accs[(e, qb)]
                if busy:
                    a0 = jnp.concatenate([y_s[1 - e][zero + AC0], acc[0:8, 128:]], axis=1)
                    acc = jnp.concatenate([a0, acc[8:]], axis=0)
                acc = acc + pv
            accs[(e, qb)] = acc
            if c < NC - 1 and (prep[n + 1] or puts):
                y_s[1 - e][AC0] = acc[0:8, 0:128]
            if n == len(items) - 1:
                acc_s[...] = acc
            elif c == NC - 1:
                finish(j, e, qb, acc)

        for n, (e, qb, c) in enumerate(items):
            if c == 0:
                qw = q_window(j, e, slice(qb * TQ, (qb + 1) * TQ))
            pieces = [key_piece(e, c, npc - 1 - t) for t in range(npc)]
            s = jnp.dot(_as_bf16(jnp.concatenate(pieces, axis=0)), qw, preferred_element_type=F32)
            pm = jnp.exp2(jnp.concatenate([s[16 * (npc - 1 - t):16 * (npc - t)] for t in range(npc)], axis=0))
            if n:
                accumulate(n - 1, p)
            else:
                jp = jnp.maximum(j - 1, 0)
                finish(jp, 1, NQ - 1, acc_s[...])
            p = jnp.concatenate([pm] + [jnp.concatenate([scores[(n, g, l)] for l in range(NL)], axis=1) for g in range(VG)], axis=0)
        accumulate(len(items) - 1, p)
        return carry

    def shifted_pair(t, carry):
        j, qb = t // NQ, t % NQ
        cols = pl.ds(pl.multiple_of(qb * TQ, TQ), TQ)
        outs = []
        for e in range(2):
            qw = q_window(j, e, cols)

            def scores(c):
                return jnp.dot(k_window(j, e, pl.ds(pl.multiple_of(c * 128, 128), 128)), qw, preferred_element_type=F32)

            def max_body(c, m):
                return jnp.maximum(m, jnp.max(scores(c), axis=0, keepdims=True))
            m = lax.fori_loop(0, NC, max_body, jnp.full((1, TQ), -jnp.inf, F32))

            def pv_body(c, acc):
                p = jnp.exp2(scores(c) - m).astype(BF16)
                return acc + jnp.dot(v_window(j, e, pl.ds(pl.multiple_of(c * 128, 128), 128)), p, preferred_element_type=F32)
            acc = lax.fori_loop(0, NC, pv_body, jnp.zeros((24, TQ), F32))
            outs.append(acc * (1.0 / (acc[23:24] if e == 0 else acc[0:1])))
        mid = jnp.where(subq < 4, outs[0][16:24], outs[1][0:8])
        ot_s[j, :, cols] = jnp.concatenate([outs[0][0:16], mid, outs[1][8:24]], axis=0)
        return carry

    acc_s[...] = jnp.ones(acc_s.shape, F32)
    lax.fori_loop(0, NP, unshifted_pair, 0)
    finish(NP - 1, 1, NQ - 1, acc_s[...])
    safe = ((jnp.max(chk_s[0], (0, 1)) <= 1.0 / L_MIN) & (jnp.min(chk_s[1], (0, 1)) >= 1.0 / L_MAX)
            & (jnp.abs(jnp.sum(chk_s[2], (0, 1))) <= O_MAX))

    @pl.when(jnp.min(jnp.where(safe, 1.0, 0.0)) < 1.0)
    def _():
        lax.fori_loop(0, NP * NQ, shifted_pair, 0)

    def attn_jobs(t):
        def rows(l, k, r0, n):
            tok = t * TB + k * TQ + l * 128
            return rows_get(ot_s, r0, n, slice(tok, tok + 128))
        per_tile = [right_jobs(2 + t % 2, l, functools.partial(rows, l)) for l in range(NL)]
        return [job for group in zip(*per_tile) for job in group]

    def first_right(t):
        cols = lambda k: slice(t * TB + k * TQ, t * TB + (k + 1) * TQ)

        def main(i):
            v = _right_operand(i, lambda u: rows_get(ot_s, (u // 2) * KH, KH, cols(u % 2)))
            b_s[2 + t % 2][i] = _as_u32(v)
            return v

        def rest(k):
            v = rows_get(ot_s, 2 * KH, D - 2 * KH, cols(k)).astype(BF16)
            b_s[2 + t % 2][7, 64 * k:64 * k + 64] = _as_u32(v)
            return v
        return main, rest

    def residual_jobs(t, r, c):
        def job(i, k):
            rr = slice(128 * r + R * i, 128 * r + R * i + R)
            out = []
            for l in range(NL):
                v = xt_s[t][k * NL + l, rr] + c[i][k][:, 128 * l:128 * l + 128]
                xt_s[t][k * NL + l, rr] = v
                out += _registers(v)
            return out
        return [functools.partial(job, i, k) for k in range(2) for i in range(2)]

    def out_proj(t, jobs, carried):
        jobs = [[]] * (t == 0) + _spread_cost(jobs, NB - (t == 0) - 1) + [[]]
        for r in range(NB):
            right = first_right(t) if t == 0 and r == 0 else right_operands(2 + t % 2)
            c = block_product(*weight_operands(a_s, A_O + 16 * r + (0 if t else zero), KH), *right, carried + jobs[r])
            carried = residual_jobs(t, r, c)
        return carried

    def activation_jobs(t, r, c):
        def job(r0):
            act = []
            for u in range(4):
                h = c[u // 2][u % 2][r0:r0 + RP]
                b0 = 2 * R * r + R * (u // 2) + r0
                g = jnp.maximum(h + jnp.concatenate([bias_s[b0:b0 + RP, :]] * NL, axis=1), 0.0)
                act.append(g * g)
            out = []
            for i in range(7):
                v = _as_u32(_right_operand(i, lambda u: act[u]))
                c_s[t % 2][i, (R * r + r0) // 2:(R * r + r0 + RP) // 2, :] = v
                out += _registers(v)
            return out
        return [functools.partial(job, r0) for r0 in range(0, R, RP)]

    def ffn_up(t, carried):
        for r in range(NF):
            c = block_product(*weight_operands(a_s, A_1 + 16 * r + (0 if t else zero), KH), *right_operands(t % 2), carried)
            carried = activation_jobs(t, r, c)
        for job in carried:
            job()

    def output_jobs(t, r, k, top, bot):
        def job(l):
            tile = k * NL + l
            y = jnp.concatenate([top[:, 128 * l:128 * l + 128], bot[:, 128 * l:128 * l + 128]], axis=0)
            y = y + bias_s[F + 128 * r:F + 128 * r + 128, :]
            v = (xt_s[t][tile, 128 * r:128 * r + 128] + y).astype(BF16).T
            o_v[zero + (t * NB + r), tile * 128:(tile + 1) * 128, :] = v
            return _registers(_as_u32(v))
        return [functools.partial(job, l) for l in range(NL)]

    def ffn_down(t, pending, jobs):
        jobs = _spread_cost(jobs, NB - 1) + [[]]
        carried = []
        for r in range(NB):
            a, _ = weight_operands(a_s, A_2 + 7 * (F // 256) * r + (0 if t else zero), F // 2)
            c = block_product(a, None, lambda i: _as_bf16(c_s[t % 2][i]), None,
                              _interleave(_spread(carried, 5) + [[], []], _spread(jobs[r], 7)), functools.partial(output_jobs, t, r, 0))
            for cp in pending:
                cp.start()
            carried = output_jobs(t, r, 1, c[0][1], c[1][1])
            pending = [cp_o[t][r]]
        return carried, pending

    carried = out_proj(1, norm_block(0, False), out_proj(0, attn_jobs(1), []))
    pending = []
    for t in range(NT):
        ffn_up(t, carried)
        carried, pending = ffn_down(t, pending, norm_block(t + 1, False) if t + 1 < NT else [])
    for job in carried:
        job()
    for cp in pending:
        cp.start()
    for row in cp_o:
        for cp in row:
            cp.wait()


@jax.jit
def pallas_sequential_preLN__softmax_full_mha__dense_activation_squared_relu__prompt_kernel(
    A_x: jax.Array,
    A_wqkv: jax.Array,
    A_wo: jax.Array,
    B_x: jax.Array,
    B_w1: jax.Array,
    B_b1: jax.Array,
    B_w2: jax.Array,
    B_b2: jax.Array,
):
    del B_x
    _, S, D = A_x.shape
    F = B_w1.shape[1]
    assert A_x.shape == (1, 2 * TB, 640) and F == 1536
    Dh, NP, NB, NC, NT = D // HEADS, HEADS // 2, D // 128, S // 128, S // TB
    heads = pltpu.VMEM((NP, 2 * Dh, S), F32)
    hbm, vmem = pl.BlockSpec(memory_space=pl.ANY), pl.BlockSpec(memory_space=pltpu.VMEM)
    return pl.pallas_call(
        _kernel,
        out_shape=jax.ShapeDtypeStruct(A_x.shape, A_x.dtype),
        in_specs=[pl.BlockSpec(memory_space=pltpu.SMEM), hbm, hbm, hbm, hbm, vmem, hbm, vmem],
        out_specs=hbm,
        scratch_shapes=[
            pltpu.VMEM((S, D), BF16), pltpu.VMEM((D, 3 * D), BF16), pltpu.VMEM((D, D), BF16),
            pltpu.VMEM((D, F), BF16), pltpu.VMEM((F, D), BF16), pltpu.VMEM((NT * NB, TB, 128), BF16),
            [pltpu.VMEM((2 * NL, D, 128), F32)] * NT,
            heads, heads, heads, heads,
            pltpu.VMEM((NP, 2 * Dh, 8 * VG * NC), F32),
            [pltpu.VMEM((VG * NC * Dh + 8 * NC + 64 + 1, 8, 128), F32)] * 2,
            [pltpu.VMEM((16 * 8, R // 2, 128), U32)] * 2,
            pltpu.VMEM((16 * NB + 16 * (F // (2 * R)) + 7 * NB * (F // 256), R // 2, 128), U32),
            [pltpu.VMEM((8, 128, TQ), U32)] * 4,
            [pltpu.VMEM((7, F // 4, TQ), U32)] * 2,
            pltpu.VMEM((F + D, 128), F32), pltpu.VMEM((3, NP, 2 * (S // TQ), 8, 128), F32), pltpu.VMEM((24, TQ), F32),
            pltpu.SemaphoreType.DMA((2 * NL + 1,)), pltpu.SemaphoreType.DMA((len(W_CUTS) - 1,)),
            pltpu.SemaphoreType.DMA((3 + NT * NB,)),
        ],
        compiler_params=pltpu.CompilerParams(vmem_limit_bytes=110 * 2**20),
    )(jnp.zeros((1,), jnp.int32), A_x, A_wqkv, A_wo, B_w1, B_b1, B_w2, B_b2)
```

```python
import functools

import jax
import jax.experimental.pallas as pl
import jax.experimental.pallas.tpu as pltpu
import jax.numpy as jnp
from jax import lax

F32, BF16, U32 = jnp.float32, jnp.bfloat16, jnp.uint32
HEADS = 32
EPS = 1e-5
LOG2E = 1.4426950408889634
L_MIN, L_MAX, O_MAX = 2.0 ** -60, 2.0 ** 100, 2.0 ** 120

TQ = 512
TB = 2 * TQ
NL = TQ // 128
R = 64
RP = 16
VG = 2
SEG = 4
PAD = 4
W_CUTS = (0, 2, 7, 15)
LN_AT = 6


def _as_bf16(x):
    return pltpu.bitcast(x, BF16)


def _as_u32(x):
    return pltpu.bitcast(x, U32)


def _spread(jobs, n):
    cut = [(i * len(jobs)) // n for i in range(n + 1)]
    return [jobs[cut[i]:cut[i + 1]] for i in range(n)]


def _spread_cost(jobs, n):
    total, seen, out = sum(c for _, c in jobs), 0, [[] for _ in range(n)]
    for job, c in jobs:
        out[min(n - 1, (2 * seen + c) * n // (2 * total))].append(job)
        seen += c
    return out


def _interleave(a, b):
    return [job for pair in zip(a, b) for part in pair for job in part]


def _nothing():
    return []


def _registers(v):
    return [v[8 * i:8 * i + 8, 128 * k:128 * k + 128] for k in range(v.shape[1] // 128) for i in range(v.shape[0] // 8)]


def _left_operand(i, blk):
    f = lambda u: blk(u).astype(F32)
    return (lambda: (f(0) + f(3)).astype(BF16), lambda: (f(2) + f(3)).astype(BF16), lambda: blk(0), lambda: blk(3),
            lambda: (f(0) + f(1)).astype(BF16), lambda: (f(2) - f(0)).astype(BF16), lambda: (f(1) - f(3)).astype(BF16))[i]()


def _right_operand(i, blk):
    return (lambda: blk(0) + blk(3), lambda: blk(0), lambda: blk(1) - blk(3), lambda: blk(2) - blk(0),
            lambda: blk(3), lambda: blk(0) + blk(1), lambda: blk(2) + blk(3))[i]().astype(BF16)


def _kernel(z_ref, x_hbm, wqkv_hbm, wo_hbm, w1_hbm, b1_ref, w2_hbm, b2_ref, o_hbm,
            x_v, wqkv_v, wo_v, w1_v, w2_v, o_v, xt_s, qt_s, kt_s, vt_s, ot_s, kv_s, y_s, aq_s, a_s, b_s, c_s,
            bias_s, chk_s, acc_s, sem_x, sem_w, sems):
    S, D = x_v.shape
    F = w1_v.shape[1]
    Dh = D // HEADS
    NP, NB, NC, NQ, NT, NF = HEADS // 2, D // 128, S // 128, S // TQ, S // TB, F // (2 * R)
    KH = (D // 256) * 128
    NG = VG * NC
    KB0, KW0 = 0, NG * Dh
    PV0 = KW0 + NC * 8
    AC0 = y_s[0].shape[0] - 1
    A_O, A_1 = 0, 16 * NB
    A_2 = A_1 + 16 * NF

    zero = z_ref[0]
    sub = lax.broadcasted_iota(jnp.int32, (8, 128), 0)
    lane = lax.broadcasted_iota(jnp.int32, (8, 128), 1)
    always = (sub + zero) >= 0
    products = []

    x_cuts = [128 * i for i in range(2 * NL + 1)] + [S]
    cp_x = [pltpu.make_async_copy(x_hbm.at[0, pl.ds(a, b - a)], x_v.at[pl.ds(a, b - a)], sem_x.at[i])
            for i, (a, b) in enumerate(zip(x_cuts, x_cuts[1:]))]
    cp_w = [pltpu.make_async_copy(wqkv_hbm.at[:, pl.ds(128 * a, 128 * (b - a))], wqkv_v.at[:, pl.ds(128 * a, 128 * (b - a))], sem_w.at[i])
            for i, (a, b) in enumerate(zip(W_CUTS, W_CUTS[1:]))]
    cp_tail = [pltpu.make_async_copy(src, dst, sems.at[i]) for i, (src, dst) in enumerate(((wo_hbm, wo_v), (w1_hbm, w1_v), (w2_hbm, w2_v)))]
    cp_o = [[pltpu.make_async_copy(o_v.at[t * NB + r], o_hbm.at[0, pl.ds(t * TB, TB), pl.ds(r * 128, 128)], sems.at[3 + t * NB + r])
             for r in range(NB)] for t in range(NT)]

    def rows_get(ref, r0, n, cols):
        return jnp.concatenate([ref[i // 5, 8 * (i % 5):8 * (i % 5) + 8, cols] for i in range(r0 // 8, (r0 + n) // 8)], axis=0)

    def rows_put(ref, r0, val, cols):
        for k in range(val.shape[0] // 8):
            i = r0 // 8 + k
            ref[i // 5, 8 * (i % 5):8 * (i % 5) + 8, cols] = val[8 * k:8 * k + 8]

    def after(val, jobs):
        deps = [pltpu.bitcast(v, val.dtype) for job in jobs for v in job()]
        if not deps:
            return val
        nr = val.shape[0] // 8
        tiles = _registers(val)
        for i, vs in enumerate(_spread(deps, len(tiles))[::-1]):
            for v in vs:
                tiles[i] = jnp.where(always, tiles[i], v)
        return jnp.concatenate([jnp.concatenate(tiles[i::nr], axis=1) for i in range(nr)], axis=0)

    def block_product(a, ar, b, br, jobs, half_done=None):
        js = iter(_spread(list(jobs), 7 if ar is None else 11))

        def mm(l, r):
            v = jnp.dot(l, r, preferred_element_type=F32)
            out = after(v, next(js))
            products.append(v[0:8, 0:128])
            return out
        rest = (lambda c, i, k: c) if ar is None else (lambda c, i, k: c + mm(ar(i), br(k)))
        m = lambda i: mm(a(i), b(i))
        m1 = m(0)
        m4 = m(3)
        m5 = m(4)
        c11 = rest(m1 + m4 - m5 + m(6), 0, 0)
        m2 = m(1)
        c21 = rest(m2 + m4, 1, 0)
        if half_done is not None:
            left = list(js)
            js = iter([x + y for x, y in zip(left, _spread(half_done(c11, c21), len(left)))])
        m3 = m(2)
        c12 = rest(m3 + m5, 0, 1)
        c22 = rest(m1 - m2 + m3 + m(5), 1, 1)
        return [[c11, c12], [c21, c22]]

    def weight_jobs(a_ref, base, kh, nrest, load):
        nk = kh // 128
        memo = []

        def blk(u):
            if not memo:
                wt = load().T
                memo.extend((wt[0:R], wt[R:2 * R]))
            return memo[u // 2][:, (u % 2) * kh:(u % 2 + 1) * kh]

        def main(i):
            v = _as_u32(_left_operand(i, blk))
            for k in range(nk):
                a_ref[zero + (base + i * nk + k), 0:R // 2] = v[:, 128 * k:128 * k + 128]
            return _registers(v)[3::4]

        def rest(i):
            blk(0)
            v = _as_u32(memo[i][:, 2 * kh:])
            a_ref[zero + (base + 7 * nk + i), 0:R // 2] = v
            return _registers(v)[-1:]
        return [functools.partial(main, i) for i in range(7)] + [functools.partial(rest, i) for i in range(nrest)]

    def weight_operands(a_ref, base, kh):
        nk = kh // 128
        a = lambda i: _as_bf16(jnp.concatenate([a_ref[base + i * nk + k, 0:R // 2] for k in range(nk)], axis=1))
        return a, (lambda i: _as_bf16(a_ref[base + 7 * nk + i, 0:R // 2]))

    def right_jobs(slot, l, rows):
        def main(r0):
            blk = [rows(u % 2, (u // 2) * KH + r0, RP) for u in range(4)]
            out = []
            for i in range(7):
                v = _as_u32(_right_operand(i, lambda u: blk[u]))
                b_s[slot][zero + i, r0 // 2:(r0 + RP) // 2, 128 * l:128 * l + 128] = v
                out += _registers(v)
            return out[4:]

        def rest(k):
            v = _as_u32(rows(k, 2 * KH, D - 2 * KH).astype(BF16))
            b_s[slot][zero + 7, 64 * k:64 * k + 64, 128 * l:128 * l + 128] = v
            return _registers(v)[-1:]
        return [(functools.partial(main, r0), 7) for r0 in range(0, KH, RP)] + [(functools.partial(rest, k), 7) for k in range(2)]

    def right_operands(slot):
        return (lambda i: _as_bf16(b_s[slot][i])), (lambda k: _as_bf16(b_s[slot][7, 64 * k:64 * k + 64]))

    def norm_jobs(t, l, from_x):
        tile = [k * NL + l for k in range(2)]
        mean, rstd, part = {}, {}, {}

        def add_up(key, v):
            v = [v[8 * i:8 * i + 8] for i in range(v.shape[0] // 8)] + ([part[key]] if key in part else [])
            while len(v) > 1:
                v = [v[i] + v[i + 1] for i in range(0, len(v) - 1, 2)] + v[len(v) - len(v) % 2:]
            part[key] = v[0]
            return v

        def mean_job(k, b):
            rr = slice(128 * b, 128 * b + 128)
            if from_x:
                v = x_v[t * TB + tile[k] * 128:t * TB + (tile[k] + 1) * 128, rr].T.astype(F32)
                xt_s[t][zero + tile[k], rr] = v
            else:
                v = after(xt_s[t][tile[k], rr], [lambda: products[-1:]])
            out = add_up(("sum", k), v)
            if b == NB - 1:
                mean[k] = jnp.broadcast_to(jnp.sum(out[0], axis=0, keepdims=True) * (1.0 / D), (8, 128))
                out = [mean[k]]
            return out

        def centered(k, r0, n):
            return (xt_s[t][zero + tile[k], r0:r0 + n].reshape(n // 8, 8, 128) - mean[k][None]).reshape(n, 128)

        def var_job(k, b):
            d = centered(k, 128 * b, 128)
            out = add_up(("var", k), d * d)
            if b == NB - 1:
                rstd[k] = jnp.broadcast_to(lax.rsqrt(jnp.sum(out[0], axis=0, keepdims=True) * (1.0 / D) + EPS), (8, 128))
                out = [rstd[k]]
            return out

        def rows(k, r0, n):
            return (centered(k, r0, n).reshape(n // 8, 8, 128) * rstd[k][None]).reshape(n, 128)
        costs = ((mean_job, 10 if from_x else 2), (var_job, 5))
        return [(functools.partial(job, k, b), cost) for job, cost in costs for k in range(2) for b in range(NB)] + right_jobs(t % 2, l, rows)

    def norm_block(t, from_x):
        per_tile = [norm_jobs(t, l, from_x) for l in range(NL)]
        passes = lambda l, i: (per_tile[l][:2 * NB], per_tile[l][2 * NB:4 * NB], per_tile[l][4 * NB:])[i] if 0 <= l < NL else []
        return [job for step in range(NL + 2) for group in zip(*[_spread(passes(step - i, i), 2 * NB) for i in range(3)])
                for jobs in group for job in jobs]

    def w2_columns(r):
        w = w2_v[:, 128 * r:128 * r + 128]
        return jnp.concatenate([w[2 * R * q + R * i:2 * R * q + R * (i + 1)] for i in range(2) for q in range(NF)], axis=0)

    def bias_job(ref, base, r):
        bias = ref[...].astype(F32).reshape(1, ref.shape[0])
        v = jnp.broadcast_to(bias[:, 128 * r:128 * r + 128], (128, 128)).T
        bias_s[base + 128 * r:base + 128 * r + 128, :] = v
        return _registers(v)[-1:]

    columns = lambda ref, r: lambda: ref[:, 128 * r:128 * r + 128]
    qkv_jobs = [weight_jobs(aq_s[r % 2], 16 * (r // 2), KH, 2, columns(wqkv_v, r)) for r in range(3 * NB)]
    tail_jobs = [job for r in range(NB) for job in weight_jobs(a_s, A_O + 16 * r, KH, 2, columns(wo_v, r))]
    tail_jobs += [job for r in range(NF) for job in weight_jobs(a_s, A_1 + 16 * r, KH, 2, columns(w1_v, r))]
    tail_jobs += [job for r in range(NB) for job in weight_jobs(a_s, A_2 + 7 * (F // 256) * r, F // 2, 0, functools.partial(w2_columns, r))]
    tail_jobs += [functools.partial(bias_job, ref, base, r) for ref, base in ((b1_ref, 0), (b2_ref, F)) for r in range(ref.shape[0] // 128)]

    def gather_job(i):
        p, rr = i // 5, slice(8 * (i % 5), 8 * (i % 5) + 8)
        out = []
        for beta in range(NG // 16):
            acc = jnp.zeros((8, 128), F32)
            for k in range(16 // VG):
                c, lo = beta * (16 // VG) + k, 8 * VG * k
                v = kt_s[zero + p, rr, 128 * c:128 * c + 128]
                shift = (lo + 8 * VG) % 128
                v = pltpu.roll(v, shift, 1) if shift else v
                acc = jnp.where((lane >= lo) & (lane < lo + 8 * VG), v, acc)
            kv_s[p, rr, 128 * beta:128 * beta + 128] = acc
            out.append(acc)
        return out[-1:]

    def k_window(j, e, cols):
        return kt_s[j, 8 * e:8 * e + 32, cols].astype(BF16).T

    def prep_jobs(j, e):
        def kb_job(beta, d):
            r = Dh * e + d
            val = jnp.broadcast_to(kv_s[j, r:r + 1, beta * 128:beta * 128 + 128], (128, 128)).T

            def put(i):
                y_s[e][zero + (KB0 + (16 * beta + i) * Dh + d)] = val[8 * i:8 * i + 8]
                return [val[8 * i:8 * i + 8]]
            return [functools.partial(put, i) for i in range(16)]

        def kw_job(c):
            kw = pltpu.bitcast(k_window(j, e, slice(c * 128, (c + 1) * 128)), F32)

            def put(t):
                y_s[e][zero + (KW0 + 8 * c + t), :, 0:32] = kw[8 * t:8 * t + 8]
                return []
            return [functools.partial(put, t) for t in range(8 - VG // 2)]
        a = [functools.partial(kb_job, beta, d) for beta in range(NG // 16) for d in range(Dh)]
        return [job for c, x in enumerate(_spread(a, NC)) for job in [functools.partial(kw_job, c)] + x]

    for l in range(NL):
        cp_x[l].start()
        cp_x[NL + l].start()
    cp_w[0].start()
    later = []
    for l in range(NL):
        for c in ([], [cp_w[1]], [], [cp_w[2]])[l]:
            c.start()
        cp_x[l].wait()
        cp_x[NL + l].wait()
        jobs = [job for job, _ in norm_jobs(0, l, True)]
        for job in jobs[:2 * NB] + later:
            job()
        later = jobs[2 * NB:]
    cp_x[2 * NL].start()
    cp_w[0].wait()
    for job in qkv_jobs[0] + later:
        job()

    def dma_job(waits, starts):
        for c in starts:
            c.start()
        for c in waits:
            c.wait()
        return []

    def qkv_store(t, r, i, k, v):
        if r < NB:
            v = v * (Dh ** -0.5 * LOG2E)
        elif r >= 2 * NB:
            v = v.astype(BF16).astype(F32)
        rows_put((qt_s, kt_s, vt_s)[r // NB], 128 * (r % NB) + R * i, v, slice(t * TB + k * TQ, t * TB + (k + 1) * TQ))
        return _registers(v)[7::8]

    side = [qkv_jobs[1:] + [[]], _spread(tail_jobs, 3 * NB)]
    for r, jobs in enumerate(_spread_cost(norm_block(1, True), 3 * NB - LN_AT - 1)):
        side[0][LN_AT + r] = _interleave(_spread(side[0][LN_AT + r], 3), _spread(jobs, 3))
    last = [functools.partial(gather_job, i) for i in range(D // 8)]
    first_head = [lambda job=job: [v for put in job() for v in put()][-1:] for job in prep_jobs(zero, 0)]
    for r, jobs in enumerate(_spread(last[:8] + _interleave(_spread(last[8:], 8), _spread(first_head, 8)), 2 * NB - 1)):
        side[1][NB + 1 + r] = side[1][NB + 1 + r] + jobs
    dmas = {(0, W_CUTS[1] - 1): [_nothing] * 2 + [functools.partial(dma_job, [cp_w[1]], [])],
            (0, LN_AT): [_nothing, functools.partial(dma_job, [cp_w[2], cp_x[2 * NL]], cp_tail)],
            (1, 0): [_nothing] * 4 + [functools.partial(dma_job, cp_tail, [])]}
    orders = (range(3 * NB), [*range(NB, 2 * NB), *range(NB), *range(2 * NB, 3 * NB)])
    carried = []
    for t in range(NT):
        for step, r in enumerate(orders[t]):
            jobs = dmas.get((t, step), []) + _interleave(_spread(carried, 4), _spread(side[t][step], 4))
            c = block_product(*weight_operands(aq_s[r % 2], 16 * (r // 2) + (0 if t else zero), KH), *right_operands(t % 2), jobs)
            carried = [functools.partial(qkv_store, t, r, i, k, c[i][k]) for k in range(2) for i in range(2)]
    for job in carried:
        job()

    subq = lax.broadcasted_iota(jnp.int32, (8, TQ), 0)
    row32 = lax.broadcasted_iota(jnp.int32, (32, TQ), 0)

    def q_window(j, e, cols):
        qw = qt_s[j, 8 * e:8 * e + 32, cols]
        return jnp.where(row32 < Dh if e == 0 else row32 >= 32 - Dh, qw, 0.0).astype(BF16)

    def v_window(j, e, cols):
        if e == 0:
            pieces = [vt_s[j, 0:8, cols], vt_s[j, 8:16, cols], jnp.where(sub < 4, vt_s[j, 16:24, cols], 1.0)]
        else:
            pieces = [jnp.where(sub >= 4, vt_s[j, 16:24, cols], 1.0), vt_s[j, 24:32, cols], vt_s[j, 32:40, cols]]
        return jnp.concatenate(pieces, axis=0)

    def finish(j, e, qb, acc):
        cols = slice(qb * TQ, (qb + 1) * TQ)
        inv = 1.0 / (acc[23:24] if e == 0 else acc[0:1])
        o = acc * inv
        inv8 = jnp.broadcast_to(inv, (8, TQ))
        for i, (f, v) in enumerate(((jnp.maximum, inv8), (jnp.minimum, inv8), (jnp.add, o))):
            chk_s[i, j, e * NQ + qb] = functools.reduce(f, _registers(v))
        if e == 0:
            ot_s[j, 0:Dh, cols] = o[0:Dh]
        else:
            ot_s[j, Dh:24, cols] = o[4:8]
            ot_s[j, 24:40, cols] = o[8:24]

    def unshifted_pair(j, carry):
        jn = jnp.minimum(j + 1, NP - 1)
        items = [(e, qb, c) for e in range(2) for qb in range(NQ) for c in range(NC)]
        prep = []
        for pj, pe in ((j, 1), (jn, 0)):
            prep += _spread(prep_jobs(pj, pe), NQ * NC - PAD) + [[] for _ in range(PAD)]
        scores, accs, puts, slot = {}, {}, [], {}
        npc = 8 - VG // 2
        cuts = [(Dh * i) // SEG for i in range(SEG + 1)]
        work = iter(_spread([(n, l, cuts[i], cuts[i + 1]) for n in range(len(items)) for l in range(NL) for i in range(SEG)], npc * len(items)))

        def key_piece(e, c, t):
            for n, l, d0, d1 in next(work):
                ne, nqb, nc = items[n]
                for g in range(VG):
                    acc = scores.get((n, g, l))
                    for d in range(d0, d1):
                        r = Dh * ne + d
                        q = jnp.broadcast_to(qt_s[j, r:r + 1, nqb * TQ + l * 128:nqb * TQ + (l + 1) * 128], (8, 128))
                        term = y_s[ne][KB0 + (VG * nc + g) * Dh + d] * q
                        acc = term if acc is None else acc + term
                    scores[(n, g, l)] = jnp.exp2(acc) if d1 == Dh else acc
                for g in range(VG):
                    y_s[e][slot.setdefault((n, g, l), PV0 + len(slot) % (AC0 - PV0))] = scores[(n, g, l)]
            return y_s[e][zero + (KW0 + c * 8 + t), :, 0:32]

        def accumulate(n, p):
            e, qb, c = items[n]
            pv = jnp.dot(v_window(j, e, slice(c * 128, (c + 1) * 128)), p, preferred_element_type=F32)
            busy = bool(prep[n] or puts)
            while puts:
                puts.pop(0)()
            for job in prep[n]:
                todo = job()
                todo.pop(0)()
                puts.extend(todo)
            if c == 0:
                acc = pv
            else:
                acc = accs[(e, qb)]
                if busy:
                    a0 = jnp.concatenate([y_s[1 - e][zero + AC0], acc[0:8, 128:]], axis=1)
                    acc = jnp.concatenate([a0, acc[8:]], axis=0)
                acc = acc + pv
            accs[(e, qb)] = acc
            if c < NC - 1 and (prep[n + 1] or puts):
                y_s[1 - e][AC0] = acc[0:8, 0:128]
            if n == len(items) - 1:
                acc_s[...] = acc
            elif c == NC - 1:
                finish(j, e, qb, acc)

        for n, (e, qb, c) in enumerate(items):
            if c == 0:
                qw = q_window(j, e, slice(qb * TQ, (qb + 1) * TQ))
            pieces = [key_piece(e, c, npc - 1 - t) for t in range(npc)]
            s = jnp.dot(_as_bf16(jnp.concatenate(pieces, axis=0)), qw, preferred_element_type=F32)
            pm = jnp.exp2(jnp.concatenate([s[16 * (npc - 1 - t):16 * (npc - t)] for t in range(npc)], axis=0))
            if n:
                accumulate(n - 1, p)
            else:
                jp = jnp.maximum(j - 1, 0)
                finish(jp, 1, NQ - 1, acc_s[...])
            p = jnp.concatenate([pm] + [jnp.concatenate([scores[(n, g, l)] for l in range(NL)], axis=1) for g in range(VG)], axis=0)
        accumulate(len(items) - 1, p)
        return carry

    def shifted_pair(t, carry):
        j, qb = t // NQ, t % NQ
        cols = pl.ds(pl.multiple_of(qb * TQ, TQ), TQ)
        outs = []
        for e in range(2):
            qw = q_window(j, e, cols)

            def scores(c):
                return jnp.dot(k_window(j, e, pl.ds(pl.multiple_of(c * 128, 128), 128)), qw, preferred_element_type=F32)

            def max_body(c, m):
                return jnp.maximum(m, jnp.max(scores(c), axis=0, keepdims=True))
            m = lax.fori_loop(0, NC, max_body, jnp.full((1, TQ), -jnp.inf, F32))

            def pv_body(c, acc):
                p = jnp.exp2(scores(c) - m).astype(BF16)
                return acc + jnp.dot(v_window(j, e, pl.ds(pl.multiple_of(c * 128, 128), 128)), p, preferred_element_type=F32)
            acc = lax.fori_loop(0, NC, pv_body, jnp.zeros((24, TQ), F32))
            outs.append(acc * (1.0 / (acc[23:24] if e == 0 else acc[0:1])))
        mid = jnp.where(subq < 4, outs[0][16:24], outs[1][0:8])
        ot_s[j, :, cols] = jnp.concatenate([outs[0][0:16], mid, outs[1][8:24]], axis=0)
        return carry

    acc_s[...] = jnp.ones(acc_s.shape, F32)
    lax.fori_loop(0, NP, unshifted_pair, 0)
    finish(NP - 1, 1, NQ - 1, acc_s[...])
    safe = ((jnp.max(chk_s[0], (0, 1)) <= 1.0 / L_MIN) & (jnp.min(chk_s[1], (0, 1)) >= 1.0 / L_MAX)
            & (jnp.abs(jnp.sum(chk_s[2], (0, 1))) <= O_MAX))

    @pl.when(jnp.min(jnp.where(safe, 1.0, 0.0)) < 1.0)
    def _():
        lax.fori_loop(0, NP * NQ, shifted_pair, 0)

    def attn_jobs(t):
        def rows(l, k, r0, n):
            tok = t * TB + k * TQ + l * 128
            return rows_get(ot_s, r0, n, slice(tok, tok + 128))
        per_tile = [right_jobs(2 + t % 2, l, functools.partial(rows, l)) for l in range(NL)]
        return [job for group in zip(*per_tile) for job in group]

    def first_right(t):
        cols = lambda k: slice(t * TB + k * TQ, t * TB + (k + 1) * TQ)

        def main(i):
            v = _right_operand(i, lambda u: rows_get(ot_s, (u // 2) * KH, KH, cols(u % 2)))
            b_s[2 + t % 2][i] = _as_u32(v)
            return v

        def rest(k):
            v = rows_get(ot_s, 2 * KH, D - 2 * KH, cols(k)).astype(BF16)
            b_s[2 + t % 2][7, 64 * k:64 * k + 64] = _as_u32(v)
            return v
        return main, rest

    def residual_jobs(t, r, c):
        def job(i, k):
            rr = slice(128 * r + R * i, 128 * r + R * i + R)
            out = []
            for l in range(NL):
                v = xt_s[t][k * NL + l, rr] + c[i][k][:, 128 * l:128 * l + 128]
                xt_s[t][k * NL + l, rr] = v
                out += _registers(v)[-1:]
            return out
        return [functools.partial(job, i, k) for k in range(2) for i in range(2)]

    def out_proj(t, jobs, carried):
        jobs = [[]] * (t == 0) + _spread_cost(jobs, NB - (t == 0) - 1) + [[]]
        for r in range(NB):
            right = first_right(t) if t == 0 and r == 0 else right_operands(2 + t % 2)
            c = block_product(*weight_operands(a_s, A_O + 16 * r + (0 if t else zero), KH), *right, carried + jobs[r])
            carried = residual_jobs(t, r, c)
        return carried

    def activation_jobs(t, r, c):
        def job(r0):
            act = []
            for u in range(4):
                h = c[u // 2][u % 2][r0:r0 + RP]
                b0 = 2 * R * r + R * (u // 2) + r0
                g = jnp.maximum(h + jnp.concatenate([bias_s[b0:b0 + RP, :]] * NL, axis=1), 0.0)
                act.append(g * g)
            out = []
            for i in range(7):
                v = _as_u32(_right_operand(i, lambda u: act[u]))
                c_s[t % 2][i, (R * r + r0) // 2:(R * r + r0 + RP) // 2, :] = v
                out += _registers(v)
            return out
        return [functools.partial(job, r0) for r0 in range(0, R, RP)]

    def ffn_up(t, carried):
        for r in range(NF):
            c = block_product(*weight_operands(a_s, A_1 + 16 * r + (0 if t else zero), KH), *right_operands(t % 2), carried)
            carried = activation_jobs(t, r, c)
        for job in carried:
            job()

    def output_jobs(t, r, k, top, bot):
        def job(l):
            tile = k * NL + l
            y = jnp.concatenate([top[:, 128 * l:128 * l + 128], bot[:, 128 * l:128 * l + 128]], axis=0)
            y = y + bias_s[F + 128 * r:F + 128 * r + 128, :]
            v = (xt_s[t][tile, 128 * r:128 * r + 128] + y).astype(BF16).T
            o_v[zero + (t * NB + r), tile * 128:(tile + 1) * 128, :] = v
            return _registers(_as_u32(v))
        return [functools.partial(job, l) for l in range(NL)]

    def ffn_down(t, pending, jobs):
        jobs = _spread_cost(jobs, NB - 1) + [[]]
        carried = []
        for r in range(NB):
            a, _ = weight_operands(a_s, A_2 + 7 * (F // 256) * r + (0 if t else zero), F // 2)
            c = block_product(a, None, lambda i: _as_bf16(c_s[t % 2][i]), None,
                              _interleave(_spread(carried, 5) + [[], []], _spread(jobs[r], 7)), functools.partial(output_jobs, t, r, 0))
            for cp in pending:
                cp.start()
            carried = output_jobs(t, r, 1, c[0][1], c[1][1])
            pending = [cp_o[t][r]]
        return carried, pending

    carried = out_proj(1, norm_block(0, False), out_proj(0, attn_jobs(1), []))
    pending = []
    for t in range(NT):
        ffn_up(t, carried)
        carried, pending = ffn_down(t, pending, norm_block(t + 1, False) if t + 1 < NT else [])
    for job in carried:
        job()
    for cp in pending:
        cp.start()
    for row in cp_o:
        for cp in row:
            cp.wait()


@jax.jit
def pallas_sequential_preLN__softmax_full_mha__dense_activation_squared_relu__prompt_kernel(
    A_x: jax.Array,
    A_wqkv: jax.Array,
    A_wo: jax.Array,
    B_x: jax.Array,
    B_w1: jax.Array,
    B_b1: jax.Array,
    B_w2: jax.Array,
    B_b2: jax.Array,
):
    del B_x
    _, S, D = A_x.shape
    F = B_w1.shape[1]
    assert A_x.shape == (1, 2 * TB, 640) and F == 1536
    Dh, NP, NB, NC, NT = D // HEADS, HEADS // 2, D // 128, S // 128, S // TB
    heads = pltpu.VMEM((NP, 2 * Dh, S), F32)
    hbm, vmem = pl.BlockSpec(memory_space=pl.ANY), pl.BlockSpec(memory_space=pltpu.VMEM)
    return pl.pallas_call(
        _kernel,
        out_shape=jax.ShapeDtypeStruct(A_x.shape, A_x.dtype),
        in_specs=[pl.BlockSpec(memory_space=pltpu.SMEM), hbm, hbm, hbm, hbm, vmem, hbm, vmem],
        out_specs=hbm,
        scratch_shapes=[
            pltpu.VMEM((S, D), BF16), pltpu.VMEM((D, 3 * D), BF16), pltpu.VMEM((D, D), BF16),
            pltpu.VMEM((D, F), BF16), pltpu.VMEM((F, D), BF16), pltpu.VMEM((NT * NB, TB, 128), BF16),
            [pltpu.VMEM((2 * NL, D, 128), F32)] * NT,
            heads, heads, heads, heads,
            pltpu.VMEM((NP, 2 * Dh, 8 * VG * NC), F32),
            [pltpu.VMEM((VG * NC * Dh + 8 * NC + 64 + 1, 8, 128), F32)] * 2,
            [pltpu.VMEM((16 * 8, R // 2, 128), U32)] * 2,
            pltpu.VMEM((16 * NB + 16 * (F // (2 * R)) + 7 * NB * (F // 256), R // 2, 128), U32),
            [pltpu.VMEM((8, 128, TQ), U32)] * 4,
            [pltpu.VMEM((7, F // 4, TQ), U32)] * 2,
            pltpu.VMEM((F + D, 128), F32), pltpu.VMEM((3, NP, 2 * (S // TQ), 8, 128), F32), pltpu.VMEM((24, TQ), F32),
            pltpu.SemaphoreType.DMA((2 * NL + 1,)), pltpu.SemaphoreType.DMA((len(W_CUTS) - 1,)),
            pltpu.SemaphoreType.DMA((3 + NT * NB,)),
        ],
        compiler_params=pltpu.CompilerParams(vmem_limit_bytes=110 * 2**20),
    )(jnp.zeros((1,), jnp.int32), A_x, A_wqkv, A_wo, B_w1, B_b1, B_w2, B_b2)
```
